```python
import os as _os
_os.environ.setdefault("JAX_PLATFORMS", "cpu")
import jax
import jax.numpy as jnp

def _softmax(x, axis=-1):
    return jax.nn.softmax(x, axis=axis)
def _gelu(x):
    return jax.nn.gelu(x, approximate=True)
def _silu(x):
    return jax.nn.silu(x)
def _sigmoid(x):
    return jax.nn.sigmoid(x)
def _layernorm(x, axis=-1, eps=1e-5):
    m = jnp.mean(x, axis=axis, keepdims=True)
    v = jnp.var(x, axis=axis, keepdims=True)
    return (x - m) / jnp.sqrt(v + eps)
def _scatter_add(tgt, idx, src, axis=0):
    return tgt.at[idx].add(src)
def _segment_sum(src, seg, n):
    return jax.ops.segment_sum(src, seg, n)
class _Rng:
    def __init__(self, key):
        self._k = key
    def _next(self):
        self._k, sub = jax.random.split(self._k)
        return sub
    def normal(self, shape):
        return jax.random.normal(self._next(), shape, dtype=jnp.bfloat16)
    def randint(self, lo, hi, shape):
        return jax.random.randint(self._next(), shape, lo, hi, dtype=jnp.int32)
    def uniform(self, shape, lo=0.0, hi=1.0):
        return jax.random.uniform(self._next(), shape, jnp.bfloat16, lo, hi)
    def permutation(self, n):
        return jax.random.permutation(self._next(), n)


kernel_name = 'concat_heads__softmax_full_mha__grouped_kv_mqa__prompt'

def setup_inputs():
    _rng = _Rng(jax.random.key(int.from_bytes(__import__("os").urandom(4), "little")))
    _w = (lambda a: (lambda t: t.astype(jnp.bfloat16) if jnp.issubdtype(t.dtype, jnp.floating) else t)(jnp.asarray(a)))
    def _A_setup():
        B, S, D = 1, 2048, 640
        return {
            "x": _w((lambda *s: _rng.normal(s) * 0.1)(B, S, D)),
            "wqkv": _w((lambda *s: _rng.normal(s) * 0.1)(D, 3 * D)),
            "wo": _w((lambda *s: _rng.normal(s) * 0.05)(D, D)),
        }
    _A_in = _A_setup()

    def _B_setup():
        B, S, D, H = 1, 2048, 640, 32
        Dh = D // H
        return {
            "x": _w((lambda *s: _rng.normal(s) * 0.05)(B, S, D)),
            "wq": _w((lambda *s: _rng.normal(s) * 0.4)(D, H * Dh)),
            "wk": _w((lambda *s: _rng.normal(s) * 0.4)(D, Dh)),
            "wv": _w((lambda *s: _rng.normal(s) * 0.05)(D, Dh)),
            "wo": _w((lambda *s: _rng.normal(s) * 0.05)(H * Dh, D)),
        }
    _B_in = _B_setup()

    return {
        "A_x": _A_in["x"],
        "A_wqkv": _A_in["wqkv"],
        "A_wo": _A_in["wo"],
        "B_x": _B_in["x"],
        "B_wq": _B_in["wq"],
        "B_wk": _B_in["wk"],
        "B_wv": _B_in["wv"],
        "B_wo": _B_in["wo"],
    }

def reference(A_x, A_wqkv, A_wo, B_x, B_wq, B_wk, B_wv, B_wo):
    def _A_ref(x, wqkv, wo):
        B, S, D = x.shape
        H = 32; Dh = D // H
        qkv = (lambda x, *d: x.transpose(*d))((x @ wqkv).reshape(B, S, 3, H, Dh), 2, 0, 3, 1, 4)
        q, k, v = qkv[0], qkv[1], qkv[2]
        scale = Dh ** -0.5
        scores = jnp.einsum("bhqd,bhkd->bhqk", q, k) * scale
        p = _softmax(scores, axis=-1)
        o = jnp.einsum("bhqk,bhkd->bhqd", p, v)
        return (lambda x, *d: x.transpose(*d))(o, 0, 2, 1, 3).reshape(B, S, D) @ wo

    def _B_ref(x, wq, wk, wv, wo):
        B, S, D = x.shape
        H = 32
        Dh = D // H
        q = (lambda x, *d: x.transpose(*d))((x @ wq).reshape(B, S, H, Dh), 0, 2, 1, 3)
        k = x @ wk
        v = x @ wv
        scores = jnp.einsum("bhqd,bkd->bhqk", q, k) * (Dh ** -0.5)
        p = _softmax(scores, axis=-1)
        o = jnp.einsum("bhqk,bkd->bhqd", p, v)
        return (lambda x, *d: x.transpose(*d))(o, 0, 2, 1, 3).reshape(B, S, H * Dh) @ wo

    a = _A_ref(A_x, A_wqkv, A_wo)
    b = _B_ref(B_x, B_wq, B_wk, B_wv, B_wo)
    return jnp.concatenate([a, b], axis=-1)
```

```python
import functools
import math
import jax
import jax.numpy as jnp
import jax.experimental.pallas as pl
import jax.experimental.pallas.tpu as pltpu

S = 2048
D = 640
H = 32
DH = 20
KW = 32
QT_ROWS = 648
QSCALE = (DH ** -0.5) * math.log2(math.e)
NT = (((1,), (1,)), ((), ()))
F32 = jnp.float32
BF16 = jnp.bfloat16
TQ = 512
CK = 128
NQ = S // TQ
NC = S // CK
NU = H * NQ
NJ = TQ // 128


def split16(total, n):
    q = total // 16
    return [16 * ((q * (i + 1)) // n - (q * i) // n) for i in range(n)]


def make(RK=512, NSB=8, SH=1, KV=384, GG=1, GJ=2, BLK=1, SK=2, LAG=1, V0=0, V1=32, EG=6, CPS=4, QD=2):
    def kernel(xa_hbm, wa_hbm, woa_hbm, xb_hbm, wqb_hbm, wkb_hbm, wvb_hbm, wob_hbm, o_hbm,
               xa_ref, wa_ref, woa_ref, xb_ref, wqb_ref, wkb_ref, wvb_ref, wob_ref, o_ref, isem, osem,
               wt_scr, ka_scr, kb_scr, qta, qtb, vta, vtb, ota, otb, sa, sb, kbc, qbb, zero_scr, tmp):
        def cp(src, dst, i):
            return pltpu.make_async_copy(src, dst, isem.at[i])
        c_wqb = cp(wqb_hbm, wqb_ref, 0)
        c_wkb = cp(wkb_hbm, wkb_ref, 1)
        c_wvb = cp(wvb_hbm, wvb_ref, 2)
        c_xb = cp(xb_hbm.at[0], xb_ref, 3)
        c_wa = cp(wa_hbm, wa_ref, 4)
        c_xa = cp(xa_hbm.at[0], xa_ref, 5)
        c_woa = cp(woa_hbm, woa_ref, 6)
        c_wob = cp(wob_hbm, wob_ref, 7)
        for c in (c_wkb, c_wvb, c_wqb, c_xb):
            c.start()

        zero_scr[...] = jnp.zeros((8, 128), jnp.int32)

        def qproj(x_ref, wt, qt_scr, qi):
            xq = x_ref[pl.ds(pl.multiple_of(qi * TQ, TQ), TQ), :]
            q = jax.lax.dot_general(wt_scr[wt], xq, NT, preferred_element_type=F32) * QSCALE
            qt_scr[qi, pl.ds(0, D), :] = q.astype(BF16).astype(F32)
            qt_scr[qi, pl.ds(D, QT_ROWS - D), :] = jnp.zeros((QT_ROWS - D, TQ), F32)

        c_wkb.wait()
        c_wvb.wait()
        wk = wkb_ref[...].astype(F32)
        wv = wvb_ref[...].astype(F32)
        z = lambda n: jnp.zeros((D, n), F32)
        wsm = jnp.concatenate([wk, z(16), wk, z(8), wv, wv, z(24)], axis=1).astype(BF16)
        c_wqb.wait()
        c_wa.start()
        c_xa.start()
        wt_scr[0] = wqb_ref[...].T
        c_xb.wait()
        c_woa.start()
        c_wob.start()

        def bbody(r, _):
            r0 = pl.multiple_of(r * TQ, TQ)
            kv = jnp.dot(xb_ref[pl.ds(r0, TQ), :], wsm, preferred_element_type=F32)
            k = kv[:, :2 * KW].astype(BF16)
            kb_scr[0, pl.ds(r0, TQ), :] = k[:, :KW]
            kb_scr[1, pl.ds(r0, TQ), :] = k[:, KW:]
            vtb[:, pl.ds(r0, TQ)] = kv.T[2 * KW:2 * KW + 48, :]
            qproj(xb_ref, 0, qtb, r)
            return 0
        jax.lax.fori_loop(0, NQ, bbody, 0)

        if KV:
            kk = kb_scr[0, pl.ds(0, KV), :].astype(F32)
            for d in range(DH):
                kbc[d] = jnp.broadcast_to(kk[:, d:d + 1], (KV, 128))

        c_wa.wait()
        wt_scr[1] = wa_ref[:, pl.ds(0, D)].T
        wt_scr[2] = wa_ref[:, pl.ds(2 * D, D)].T
        c_xa.wait()
        lane = jax.lax.broadcasted_iota(jnp.int32, (RK, KW), 1)

        def kvbody(r, _):
            r0 = pl.multiple_of(r * RK, RK)
            x = xa_ref[pl.ds(r0, RK), :]
            k = jnp.dot(x, wa_ref[:, pl.ds(D, D)], preferred_element_type=F32)
            for h in range(H):
                lo = 4 * (h % 2)
                w0 = DH * h - lo
                if w0 + KW <= D:
                    kw = k[:, w0:w0 + KW]
                else:
                    kw = jnp.concatenate([k[:, w0:D], jnp.zeros((RK, w0 + KW - D), F32)], axis=1)
                kh = jnp.where(jnp.logical_and(lane >= lo, lane < lo + DH), kw, 0.0)
                ka_scr[h, pl.ds(r0, RK), :] = kh.astype(BF16)
            vta[:, pl.ds(r0, RK)] = jax.lax.dot_general(wt_scr[2], x, NT, preferred_element_type=F32)
            return 0
        jax.lax.fori_loop(0, S // RK, kvbody, 0)

        def qabody(qi, _):
            qproj(xa_ref, 1, qta, qi)
            return 0
        jax.lax.fori_loop(0, NQ, qabody, 0)

        rows24k = jax.lax.broadcasted_iota(jnp.int32, (24, CK), 0)
        A = dict(qt=qta, vt=vta, ot=ota, s=sa, k=ka_scr, a=True, pieces=split16(S, NC), r0=0)
        B = dict(qt=qtb, vt=vtb, ot=otb, s=sb, k=kb_scr, a=False, pieces=split16(S - KV, NC), r0=KV)

        def uparams(u):
            if isinstance(u, int):
                h, qi = u // NQ, u % NQ
                odd = h % 2
                return h, odd, h * DH - 4 * odd, qi
            h = jax.lax.shift_right_logical(u, 2)
            odd = jax.lax.bitwise_and(h, 1)
            orow = pl.multiple_of(h * DH - 4 * odd, 8)
            return h, odd, orow, jax.lax.bitwise_and(u, NQ - 1)

        def qb_row(u, d):
            h, odd, orow, qi = uparams(u)
            t0 = d // 8 * 8
            t1 = (d + 4) // 8 * 8
            we = qtb[qi, pl.ds(orow + t0, 8), :]
            wo = qtb[qi, pl.ds(orow + t1, 8), :]
            row = jnp.where(odd == 1, wo[d + 4 - t1:d + 5 - t1, :], we[d - t0:d + 1 - t0, :])
            qbb[d] = jnp.broadcast_to(row, (8, TQ))

        def run(j, prevA, prevB, do_qk=True):
            nv1 = zero_scr[...] != 0
            never = jnp.concatenate([nv1] * NJ, axis=1)
            toks = []
            deps = []

            def qk_piece(br, w, kidx, r0, n, m8):
                k = br['k'][kidx, pl.ds(r0, n), :]
                s = jnp.dot(k, w, preferred_element_type=F32)
                br['s'][pl.ds(r0, n), :] = s
                run_m = []
                for t in range(0, n, 8):
                    st = s[t:t + 8, :]
                    m8 = st if m8 is None else jnp.maximum(m8, st)
                    run_m.append(m8)
                for i in range(NSB):
                    toks.append(run_m[((i * n) // NSB) // 8])
                return m8

            def pv_chunk(br, u, c, m, acc):
                h, odd, orow, qi = uparams(u)
                vrow = orow if br['a'] else (16 * odd if isinstance(odd, int) else pl.multiple_of(16 * odd, 8))
                SB = CK // NSB
                ps = []
                for i in range(NSB):
                    ti = len(toks) - 2 * NSB + (NSB - 1 - i) - SH
                    mi = jnp.where(never, toks[ti], m) if (ti >= 0 and toks[ti] is not None) else m
                    ps.append(jnp.exp2(br['s'][pl.ds(c * CK + i * SB, SB), :].reshape(SB // 8, 8, TQ) - mi[None]).reshape(SB, TQ))
                p = jnp.concatenate(ps, axis=0)
                v = br['vt'][pl.ds(vrow, 24), pl.ds(c * CK, CK)]
                dep = deps[-1 - LAG] if len(deps) > LAG else None
                if QD and len(deps) == 1 and do_qk and KV:
                    dep = qbb[DH - 1, :, pl.ds(TQ - 128, 128)]
                    if QD == 2:
                        for d in range(DH - 1):
                            dep = jnp.maximum(dep, qbb[d, :, pl.ds((d % NJ) * 128, 128)])
                one = jnp.ones((8, CK), F32) if dep is None else jnp.where(nv1, dep, 1.0)
                v = jnp.where(rows24k == 20 - 20 * odd, jnp.concatenate([one] * 3, axis=0), v)
                o = jnp.dot(v, p, preferred_element_type=F32)
                return o if acc is None else o + acc

            def finish(br, u, acc):
                h, odd, orow, qi = uparams(u)
                br['ot'][qi, h] = acc

            def red(m8):
                return jnp.broadcast_to(jnp.max(m8, axis=0, keepdims=True), (8, TQ))

            groups = []
            ngb = KV // 8 // GG
            npj = NJ // GJ
            for b0 in range(0, ngb, BLK):
                blk = list(range(b0, min(b0 + BLK, ngb)))
                for ps in range(npj):
                    for i, gb in enumerate(blk):
                        pj = (len(groups) + (ps if len(blk) % npj == 0 else 0)) % npj if False else (i + ps) % npj
                        groups.append([(gb * GG + a, pj * GJ + c) for a in range(GG) for c in range(GJ)])
            assert sorted(v for g_ in groups for v in g_) == [(g, jj) for g in range(KV // 8) for jj in range(NJ)]
            sched = {}
            if do_qk and KV:
                dur = [p + 24 for p in A['pieces'] + B['pieces']]
                tot = sum(dur[V0:V1])
                cum = 0
                gi = 0
                for sl in range(V0, V1):
                    cum += dur[sl]
                    while gi < len(groups) and (gi + 1) * tot <= cum * len(groups):
                        sched.setdefault(sl, []).append(gi)
                        for (g, _) in groups[gi]:
                            assert g < EG or sl > (g * 8) // CK + SK, (g, sl)
                        gi += 1
                assert gi == len(groups)
            vst = dict(dep=None, mv={})
            if do_qk and KV:
                for d in range(DH):
                    qb_row(j, d)

            def vpu_group(gi):
                grp = groups[gi]
                accs = {}
                for d in range(DH):
                    kbs = {}
                    qbs = {}
                    for (g, jj) in grp:
                        if g not in kbs:
                            kbs[g] = kbc[d, pl.ds(g * 8, 8), :]
                            if d == 0 and vst['dep'] is not None and GG <= GJ:
                                kbs[g] = jnp.where(nv1, vst['dep'], kbs[g])
                        if jj not in qbs:
                            qbs[jj] = qbb[d, :, pl.ds(jj * 128, 128)]
                            if d == 0 and vst['dep'] is not None and GG > GJ:
                                qbs[jj] = jnp.where(nv1, vst['dep'], qbs[jj])
                        t = kbs[g] * qbs[jj]
                        key = (g, jj)
                        accs[key] = t if key not in accs else accs[key] + t
                for (g, jj) in grp:
                    a = accs[(g, jj)]
                    (tmp if g < EG else sb)[pl.ds(g * 8, 8), pl.ds(jj * 128, 128)] = a
                    vst['mv'][jj] = a if jj not in vst['mv'] else jnp.maximum(vst['mv'][jj], a)
                dep = None
                for jj in sorted(set(jj for _, jj in grp)):
                    dep = vst['mv'][jj] if dep is None else jnp.maximum(dep, vst['mv'][jj])
                vst['dep'] = dep

            mB_prev = None if prevB is None else red(prevB)
            accB = None
            accA = None
            m8A = m8B = None
            for ph, br in enumerate((A, B)):
                if do_qk:
                    h, odd, orow, qi = uparams(j)
                    w = br['qt'][qi, pl.ds(orow, KW), :].astype(BF16)
                    kidx = h if br['a'] else odd
                r0 = br['r0']
                m8 = None
                for c in range(NC):
                    sl = ph * NC + c
                    if do_qk:
                        m8 = qk_piece(br, w, kidx, r0, br['pieces'][c], m8)
                        r0 += br['pieces'][c]
                        for gi in sched.get(sl, []):
                            vpu_group(gi)
                    else:
                        toks.extend([None] * NSB)
                    deps.append(vst['dep'])
                    if do_qk and KV and EG and NC <= sl < NC + EG:
                        g = sl - NC
                        sb[pl.ds(g * 8, 8), :] = jnp.where(never, toks[-NSB - 1], tmp[pl.ds(g * 8, 8), :])
                    if ph == 0:
                        if c < SK:
                            if prevA is not None:
                                prevA = (prevA[0], pv_chunk(A, j - 1, NC - SK + c, prevA[0], prevA[1]))
                                if c == SK - 1:
                                    finish(A, j - 1, prevA[1])
                        elif prevB is not None:
                            accB = pv_chunk(B, j - 1, c - SK, mB_prev, accB)
                    else:
                        if c < SK:
                            if prevB is not None:
                                accB = pv_chunk(B, j - 1, NC - SK + c, mB_prev, accB)
                                if c == SK - 1:
                                    finish(B, j - 1, accB)
                        elif do_qk:
                            accA = pv_chunk(A, j, c - SK, mA, accA)
                if ph == 0:
                    if do_qk:
                        mA = red(m8)
                else:
                    m8B = m8
            if not do_qk:
                return None
            if KV:
                m8B = jnp.maximum(m8B, jnp.concatenate([vst['mv'][jj] for jj in range(NJ)], axis=1))
            return mA, accA, m8B

        carry = run(0, None, None)

        def body(j, carry):
            mA, accA, m8B = carry
            return run(j, (mA, accA), m8B)

        mA, accA, m8B = jax.lax.fori_loop(1, NU, body, carry)
        run(NU, (mA, accA), m8B, do_qk=False)

        rows8 = jax.lax.broadcasted_iota(jnp.int32, (8, TQ), 0)

        c_woa.wait()
        c_wob.wait()

        def ocp(qi, i):
            r0 = pl.multiple_of(qi * TQ, TQ)
            return pltpu.make_async_copy(o_ref.at[i, pl.ds(r0, TQ), :],
                                         o_hbm.at[0, pl.ds(r0, TQ), pl.ds(i * D, D)], osem.at[2 * qi + i])

        def obody(qi, _):
            for i, (ot, wo_ref) in enumerate(((ota, woa_ref), (otb, wob_ref))):
                parts = []
                for hp in range(H // 2):
                    ae = ot[qi, 2 * hp]
                    ao = ot[qi, 2 * hp + 1]
                    oe = ae * (1.0 / ae[20:21, :])
                    oo = ao * (1.0 / ao[0:1, :])
                    parts += [oe[0:16], jnp.where(rows8 < 4, oe[16:24], oo[0:8]), oo[8:24]]
                o = jnp.concatenate(parts, axis=0).T.astype(BF16)
                o_ref[i, pl.ds(pl.multiple_of(qi * TQ, TQ), TQ), :] = jnp.dot(
                    o, wo_ref[...], preferred_element_type=F32).astype(o_ref.dtype)
                ocp(qi, i).start()
            return 0
        jax.lax.fori_loop(0, NQ, obody, 0)
        for qi in range(NQ):
            for i in range(2):
                ocp(qi, i).wait()

    @jax.jit
    def fn(A_x, A_wqkv, A_wo, B_x, B_wq, B_wk, B_wv, B_wo):
        ins = (A_x, A_wqkv, A_wo, B_x, B_wq, B_wk, B_wv, B_wo)
        return pl.pallas_call(
            kernel,
            in_specs=[pl.BlockSpec(memory_space=pl.ANY)] * 8,
            out_specs=pl.BlockSpec(memory_space=pl.ANY),
            out_shape=jax.ShapeDtypeStruct((1, S, 2 * D), BF16),
            scratch_shapes=[pltpu.VMEM(a.shape[-2:], a.dtype) for a in ins] + [
                pltpu.VMEM((2, S, D), BF16),
                pltpu.SemaphoreType.DMA((8,)),
                pltpu.SemaphoreType.DMA((2 * NQ,)),
                pltpu.VMEM((3, D, D), BF16),
                pltpu.VMEM((H, S, KW), BF16),
                pltpu.VMEM((2, S, KW), BF16),
                pltpu.VMEM((NQ, QT_ROWS, TQ), F32),
                pltpu.VMEM((NQ, QT_ROWS, TQ), F32),
                pltpu.VMEM((D, S), F32),
                pltpu.VMEM((48, S), F32),
                pltpu.VMEM((NQ, H, 24, TQ), F32),
                pltpu.VMEM((NQ, H, 24, TQ), F32),
                pltpu.VMEM((S, TQ), F32),
                pltpu.VMEM((S, TQ), F32),
                pltpu.VMEM((DH, max(KV, 8), 128), F32),
                pltpu.VMEM((DH, 8, TQ), F32),
                pltpu.VMEM((8, 128), jnp.int32),
                pltpu.VMEM((max(EG, 1) * 8, TQ), F32),
            ],
            compiler_params=pltpu.CompilerParams(vmem_limit_bytes=110 * 1024 * 1024),
        )(*ins)

    return fn


_impl = make()


@jax.jit
def pallas_concat_heads__softmax_full_mha__grouped_kv_mqa__prompt_kernel(
        A_x, A_wqkv, A_wo, B_x, B_wq, B_wk, B_wv, B_wo):
    return _impl(A_x, A_wqkv, A_wo, B_x, B_wq, B_wk, B_wv, B_wo)
```

```python
import math
import jax
import jax.numpy as jnp
import jax.experimental.pallas as pl
import jax.experimental.pallas.tpu as pltpu

S = 2048
D = 640
H = 32
DH = 20
HP = 24
KW = 32
QSCALE = (DH ** -0.5) * math.log2(math.e)
NT = (((1,), (1,)), ((), ()))
F32 = jnp.float32
BF16 = jnp.bfloat16
U32 = jnp.uint32
TQ = 512
CK = 128
NQ = S // TQ
NC = S // CK
NU = H * NQ
NJ = TQ // 128
TPC = TQ // CK


def make(L=128, LB=112, NV4=(4, 4, 4, 6), NE=8, PW=8, PR=16, SPAN=0.9, NFAST=0, FORCE_BAD=False, NEWTON2=False):
    NVT = tuple(NV4) * NQ
    NMT = tuple(16 - n for n in NVT)
    KV = 8 * sum(NVT)
    NB = 8 * sum(NMT)
    voff = [8 * sum(NVT[:t]) for t in range(NC + 1)]
    moff = [8 * sum(NMT[:t]) for t in range(NC + 1)]

    def kernel(xa_hbm, wa_hbm, woa_hbm, xb_hbm, wqb_hbm, wkb_hbm, wvb_hbm, wob_hbm, o_hbm,
               xa_ref, wa_ref, woa_ref, xb_ref, wqb_ref, wob_ref, o_ref, isem, xsem, osem,
               wsm_scr, ka_scr, kb_scr, kbn_scr, qta, qtb, vta, vtb, ota, otb, pc, sv, kbc, zero_scr, wkb_ref, wvb_ref, flag):
        def cp(src, dst, i):
            return pltpu.make_async_copy(src, dst, isem.at[i])

        def xb_cp(r):
            r0 = r * TQ if isinstance(r, int) else pl.multiple_of(r * TQ, TQ)
            return pltpu.make_async_copy(xb_hbm.at[0, pl.ds(r0, TQ), :], xb_ref.at[pl.ds(r0, TQ), :], xsem.at[r])
        c_wqb = cp(wqb_hbm, wqb_ref, 0)
        c_wkb = cp(wkb_hbm, wkb_ref, 1)
        c_wvb = cp(wvb_hbm, wvb_ref, 2)
        c_wa = cp(wa_hbm, wa_ref, 3)
        c_xa = cp(xa_hbm.at[0], xa_ref, 4)
        c_woa = cp(woa_hbm, woa_ref, 5)
        c_wob = cp(wob_hbm, wob_ref, 6)
        for c in (c_wkb, c_wvb, xb_cp(0), c_wqb, xb_cp(1), xb_cp(2), xb_cp(3)):
            c.start()

        zero_scr[...] = jnp.zeros((8, 128), jnp.int32)
        rows24 = jax.lax.broadcasted_iota(jnp.int32, (HP, TQ), 0)
        vfill = jnp.where(rows24 == DH, 1.0, 0.0)

        def head_rows(x, h, fill):
            if DH * h + HP <= x.shape[0]:
                w = x[DH * h:DH * h + HP]
            else:
                w = jnp.concatenate([x[DH * h:], x[:DH * h + HP - x.shape[0]]], axis=0)
            return jnp.where(rows24 < DH, w, fill)

        def kload(ref, idx, r0, n):
            return pltpu.bitcast(ref[idx, pl.ds(r0 // 2, n // 2), :], BF16)

        def qproj(x, w, qt_scr, qi):
            q = (jnp.dot(x, w, preferred_element_type=F32) * QSCALE).astype(BF16)
            qt = q.T.astype(F32)
            for h in range(H):
                qt_scr[qi, h] = head_rows(qt, h, 0.0)

        c_wkb.wait()
        c_wvb.wait()
        z = lambda n: jnp.zeros((n, D), F32)
        wsm_scr[...] = jnp.concatenate(
            [wkb_ref[...].astype(F32), z(12), wvb_ref[...].astype(F32), z(76)], axis=0).astype(BF16)
        c_wqb.wait()
        c_wa.start()
        c_xa.start()

        def bbody(r, _):
            r0 = pl.multiple_of(r * TQ, TQ)
            xb_cp(r).wait()
            x = xb_ref[pl.ds(r0, TQ), :]
            kv = jax.lax.dot_general(x, wsm_scr[...], NT, preferred_element_type=F32)
            lane = jax.lax.broadcasted_iota(jnp.int32, (TQ, 128), 1)
            k = jnp.where(lane == HP, 1.0, kv).astype(BF16).astype(F32)
            kbn_scr[pl.ds(r0, TQ), :] = k
            km = jnp.concatenate([k[t * CK + 8 * g:t * CK + 8 * g + 8, :KW] for t in range(TPC)
                                  for g in range(NMT[t] - 1, -1, -1)], axis=0).astype(BF16)
            n2 = moff[TPC] // 2
            kb_scr[0, pl.ds(pl.multiple_of(r * n2, 8), n2), :] = pltpu.bitcast(km, U32)
            vtb[0, :, pl.ds(r0, TQ)] = jnp.where(rows24 < DH, kv.T[KW:KW + HP, :], vfill)
            qproj(x, wqb_ref[...], qtb, r)
            return 0
        jax.lax.fori_loop(0, NQ, bbody, 0)

        c_woa.start()
        c_wob.start()
        c_wa.wait()
        c_xa.wait()
        lane = jax.lax.broadcasted_iota(jnp.int32, (TQ, KW), 1)

        def kvbody(r, _):
            r0 = pl.multiple_of(r * TQ, TQ)
            x = xa_ref[pl.ds(r0, TQ), :]
            k = jnp.dot(x, wa_ref[:, pl.ds(D, D)], preferred_element_type=F32)
            k = jnp.concatenate([k[t * CK + 8 * g:t * CK + 8 * g + 8] for t in range(TPC)
                                 for g in range(15, -1, -1)], axis=0)
            fill = jnp.where(lane == HP, 1.0, 0.0)
            for h in range(H):
                w0 = DH * h
                if w0 + KW <= D:
                    kw = k[:, w0:w0 + KW]
                else:
                    kw = jnp.concatenate([k[:, w0:D], jnp.zeros((TQ, w0 + KW - D), F32)], axis=1)
                kh = jnp.where(lane < DH, kw, fill).astype(BF16)
                ka_scr[h, pl.ds(pl.multiple_of(r * (TQ // 2), TQ // 2), TQ // 2), :] = pltpu.bitcast(kh, U32)
            v = jnp.dot(x, wa_ref[:, pl.ds(2 * D, D)], preferred_element_type=F32).astype(BF16)
            vt = v.T.astype(F32)
            for h in range(H):
                vta[h, :, pl.ds(r0, TQ)] = head_rows(vt, h, vfill)
            return 0
        jax.lax.fori_loop(0, NQ, kvbody, 0)

        def qabody(r, _):
            r0 = pl.multiple_of(r * TQ, TQ)
            qproj(xa_ref[pl.ds(r0, TQ), :], wa_ref[:, pl.ds(0, D)], qta, r)
            for t in range(TPC):
                kk = kbn_scr[pl.ds(r0 + t * CK + 8 * NMT[t], 8 * NVT[t]), :]
                o = pl.multiple_of(r * voff[TPC] + voff[t], 8)
                for d in range(DH):
                    kbc[d, pl.ds(o, 8 * NVT[t]), :] = jnp.broadcast_to(kk[:, d:d + 1], (8 * NVT[t], 128))
            return 0
        jax.lax.fori_loop(0, NQ, qabody, 0)

        A = dict(qt=qta, vt=vta, ot=ota, k=ka_scr, a=True)
        B = dict(qt=qtb, vt=vtb, ot=otb, k=kb_scr, a=False)

        def uparams(u):
            if isinstance(u, int):
                return u // NQ, u % NQ
            return jax.lax.shift_right_logical(u, 2), jax.lax.bitwise_and(u, NQ - 1)

        def weights(br, u, negm):
            h, qi = uparams(u)
            w = jnp.concatenate([br['qt'][qi, h], negm], axis=0).astype(BF16)
            return w, (h if br['a'] else 0)

        def probe(br, u):
            w, kidx = weights(br, u, jnp.zeros((8, TQ), F32))
            s = jnp.dot(kload(br['k'], kidx, 0, PR), w, preferred_element_type=F32)
            m = jnp.max(s, axis=0, keepdims=True)
            return jnp.broadcast_to(-m, (8, TQ)).astype(BF16).astype(F32)

        def qk(br, wk_, r0, n):
            w, kidx = wk_
            s = jnp.dot(kload(br['k'], kidx, r0, n), w, preferred_element_type=F32)
            p = jnp.exp2(s)
            return [p[t:t + 8] for t in range(0, n, 8)]

        def pv(br, u, t, groups, acc):
            h, qi = uparams(u)
            p = jnp.concatenate(groups[::-1], axis=0)
            v = br['vt'][h if br['a'] else 0, :, pl.ds(t * CK, CK)]
            o = jnp.dot(v, p, preferred_element_type=F32)
            return o if acc is None else o + acc

        groups = []
        nblk = KV // 48
        assert nblk * 48 == KV
        for bi in range(nblk):
            for (ab, c) in ((0, 0), (1, 3), (0, 1), (1, 0), (0, 2), (1, 1), (0, 3), (1, 2)):
                groups.append([(bi * 6 + ab * 3 + a, c) for a in range(3)])
        NG = len(groups)
        pos = [L] + [CK * (t + 1) + L for t in range(NC)] + [S + moff[t + 1] + LB for t in range(NC - 1)] + [S + NB + L]
        dur = [pos[i + 1] - pos[i] + 24 for i in range(2 * NC)]
        tot = sum(dur)
        gwin = []
        for gi in range(NG):
            if gi < NE:
                gwin.append(-1)
                continue
            tgt = int((gi - NE) * tot * SPAN) // (NG - NE)
            cum, w = 0, 0
            while cum + dur[w] <= tgt:
                cum += dur[w]
                w += 1
            gwin.append(w)
        for gi in range(NG):
            for (g, _) in groups[gi]:
                t = max(i for i in range(NC) if voff[i] <= 8 * g)
                assert gwin[gi] <= NC + t, (gi, gwin[gi], t)
                assert gwin[gi] + 2 * NC > NC + t

        def vpu_group(gi, u, nm, nv1, dep):
            h, qi = uparams(u)
            g0, jj = groups[gi][0]
            init = nm[:, jj * 128:(jj + 1) * 128]
            if dep is not None:
                init = jnp.where(nv1, jnp.maximum(jnp.maximum(dep[0:8], dep[8:16]), dep[16:24]), init)
            acc = jnp.concatenate([init] * 3, axis=0)
            for d in range(DH):
                acc = acc + kbc[d, pl.ds(g0 * 8, 24), :] * qtb[qi, h, pl.ds(d, 1), pl.ds(jj * 128, 128)]
            sv[pl.ds(g0 * 8, 24), pl.ds(jj * 128, 128)] = acc
            return acc

        def body(j, carry):
            nmA, nmB = carry
            jn = jnp.minimum(j + 1, NU - 1)
            nv1 = zero_scr[...] != 0
            wA = weights(A, j, nmA)
            wB = weights(B, j, nmB)
            stream = [pc[pl.ds(t, 8), :] for t in range(0, L, 8)]
            acc = None
            dep = None
            for w in range(2 * NC):
                a, b = pos[w], pos[w + 1]
                for (lo, hi, br, wk_) in ((0, S, A, 'A'), (S, S + NB, B, 'B'), (S + NB, S + NB + L, A, 'N')):
                    x0, x1 = max(a, lo), min(b, hi)
                    if x0 < x1:
                        if wk_ == 'N' and x0 == lo:
                            wN = weights(A, jn, nmA2)
                        out = qk(br, {'A': wA, 'B': wB}.get(wk_) or wN, x0 - lo, x1 - x0)
                        if wk_ == 'N':
                            for i, g in enumerate(out):
                                pc[pl.ds(x0 - lo + 8 * i, 8), :] = g
                        else:
                            stream += out
                if w == PW:
                    nmA2 = probe(A, jn)
                if w == PW + 1:
                    nmB2 = probe(B, jn)
                for gi in range(NG):
                    if gwin[gi] == w:
                        dep = vpu_group(gi, j, nmB, nv1, dep)
                for gi in range(NG):
                    if gwin[gi] + 2 * NC == w:
                        dep = vpu_group(gi, jn, nmB2, nv1, dep)
                if w < NC:
                    acc = pv(A, j, w, stream[16 * w:16 * w + 16], acc)
                else:
                    t = w - NC
                    s0 = 16 * NC + sum(NMT[:t])
                    vg = [jnp.exp2(sv[pl.ds(voff[t] + 8 * g, 8), :]) for g in range(NVT[t] - 1, -1, -1)]
                    acc = pv(B, j, t, vg + stream[s0:s0 + NMT[t]], acc)
                if w % NC == NC - 1:
                    h, qi = uparams(j)
                    (ota if w < NC else otb)[qi, h] = acc
                    acc = None
            return nmA2, nmB2

        nmA = probe(A, 0)
        nmB = probe(B, 0)
        for i, g in enumerate(qk(A, weights(A, 0, nmA), 0, L)):
            pc[pl.ds(8 * i, 8), :] = g
        for gi in range(min(NE, NG)):
            vpu_group(gi, 0, nmB, None, None)
        jax.lax.fori_loop(0, NU, body, (nmA, nmB))

        def slow(br):
            def unit(u, _):
                h, qi = uparams(u)
                w, kidx = weights(br, u, jnp.zeros((8, TQ), F32))

                def scores(t):
                    if br['a']:
                        k = pltpu.bitcast(ka_scr[kidx, pl.ds(pl.multiple_of(t * (CK // 2), CK // 2), CK // 2), :], BF16)
                        s = jnp.dot(k, w, preferred_element_type=F32)
                        return jnp.concatenate([s[8 * g:8 * g + 8] for g in range(15, -1, -1)], axis=0)
                    k = kbn_scr[pl.ds(pl.multiple_of(t * CK, CK), CK), :][:, :KW].astype(BF16)
                    return jnp.dot(k, w, preferred_element_type=F32)

                m = jax.lax.fori_loop(
                    0, NC, lambda t, m: jnp.maximum(m, jnp.max(scores(t), axis=0, keepdims=True)),
                    jnp.full((1, TQ), -jnp.inf, F32))

                def acc_tile(t, acc):
                    p = jnp.exp2(scores(t) - m)
                    v = br['vt'][kidx, :, pl.ds(pl.multiple_of(t * CK, CK), CK)]
                    return acc + jnp.dot(v, p, preferred_element_type=F32)
                br['ot'][qi, h] = jax.lax.fori_loop(0, NC, acc_tile, jnp.zeros((HP, TQ), F32))
                return 0
            jax.lax.fori_loop(0, NU, unit, 0)

        c_woa.wait()
        c_wob.wait()

        def ocp(qi, i):
            r0 = pl.multiple_of(qi * TQ, TQ)
            return pltpu.make_async_copy(o_ref.at[i, pl.ds(r0, TQ), :],
                                         o_hbm.at[0, pl.ds(r0, TQ), pl.ds(i * D, D)], osem.at[2 * qi + i])

        def obody(qi, chk):
            lmin, lmax, bad = chk
            for i, (ot, wo_ref) in enumerate(((ota, woa_ref), (otb, wob_ref))):
                parts = []
                for h in range(H):
                    a = ot[qi, h]
                    lmin = jnp.minimum(lmin, a[16:24])
                    lmax = jnp.maximum(lmax, a[16:24])
                    l = ot[qi, h, pl.ds(DH, 1), :]
                    r = pl.reciprocal(l, approx=True)
                    r = r * (2.0 - l * r)
                    r = r * (2.0 - l * r) if NEWTON2 else r
                    parts.append((a * r)[:DH])
                o = jnp.concatenate(parts, axis=0).T.astype(BF16)
                y = jnp.dot(o, wo_ref[...], preferred_element_type=F32)
                fin = jnp.where(jnp.abs(y) < 2.0 ** 127, 0.0, 1.0)
                bad = jnp.maximum(bad, jnp.max(fin.reshape(TQ // 8, 8, D), axis=0))
                o_ref[i, pl.ds(pl.multiple_of(qi * TQ, TQ), TQ), :] = y.astype(o_ref.dtype)
                ocp(qi, i).start()
            return lmin, lmax, bad

        flag[0] = 1

        def attempt(p, _):
            @pl.when(flag[0] != 0)
            def _():
                @pl.when(p == 1)
                def _():
                    slow(A)
                    slow(B)
                one = jnp.ones((8, TQ), F32)
                lmin, lmax, bad = jax.lax.fori_loop(0, NQ, obody, (one, one, jnp.zeros((8, D), F32)))
                lok = jnp.logical_and(lmin[DH - 16:DH - 15] > 2.0 ** -16, lmax[DH - 16:DH - 15] < 2.0 ** 100)
                nbad = jnp.max(bad) + jnp.max(jnp.where(lok, 0.0, 1.0))
                flag[0] = jnp.where(nbad > (-1.0 if FORCE_BAD else 0.0), 1, 0)
                for qi in range(NQ):
                    for i in range(2):
                        ocp(qi, i).wait()
            return 0
        jax.lax.fori_loop(0, 2, attempt, 0)

    @jax.jit
    def fn(A_x, A_wqkv, A_wo, B_x, B_wq, B_wk, B_wv, B_wo):
        ins = (A_x, A_wqkv, A_wo, B_x, B_wq, B_wk.T, B_wv.T, B_wo)
        return pl.pallas_call(
            kernel,
            in_specs=[pl.BlockSpec(memory_space=pl.ANY)] * 8,
            out_specs=pl.BlockSpec(memory_space=pl.ANY),
            out_shape=jax.ShapeDtypeStruct((1, S, 2 * D), BF16),
            scratch_shapes=[pltpu.VMEM(a.shape[-2:], a.dtype) for a in ins[:5] + ins[7:]] + [
                pltpu.VMEM((2, S, D), BF16),
                pltpu.SemaphoreType.DMA((7,)),
                pltpu.SemaphoreType.DMA((NQ,)),
                pltpu.SemaphoreType.DMA((2 * NQ,)),
                pltpu.VMEM((128, D), BF16),
                pltpu.VMEM((H, S // 2, KW), U32),
                pltpu.VMEM((1, S // 2, KW), U32),
                pltpu.VMEM((S, 128), F32),
                pltpu.VMEM((NQ, H, HP, TQ), F32),
                pltpu.VMEM((NQ, H, HP, TQ), F32),
                pltpu.VMEM((H, HP, S), F32),
                pltpu.VMEM((1, HP, S), F32),
                pltpu.VMEM((NQ, H, HP, TQ), F32),
                pltpu.VMEM((NQ, H, HP, TQ), F32),
                pltpu.VMEM((L, TQ), F32),
                pltpu.VMEM((768, TQ), F32),
                pltpu.VMEM((DH, 768, 128), F32),
                pltpu.VMEM((8, 128), jnp.int32),
                pltpu.VMEM((DH, D), BF16),
                pltpu.VMEM((DH, D), BF16),
                pltpu.SMEM((1,), jnp.int32),
            ],
            compiler_params=pltpu.CompilerParams(vmem_limit_bytes=110 * 1024 * 1024),
        )(*ins)

    return fn


_impl = make()


@jax.jit
def pallas_concat_heads__softmax_full_mha__grouped_kv_mqa__prompt_kernel(
        A_x, A_wqkv, A_wo, B_x, B_wq, B_wk, B_wv, B_wo):
    return _impl(A_x, A_wqkv, A_wo, B_x, B_wq, B_wk, B_wv, B_wo)
```

```python
import math

import jax
import jax.numpy as jnp
import jax.experimental.pallas as pl
import jax.experimental.pallas.tpu as pltpu

S = 2048
D = 640
H = 32
DH = 20
HP = 24
KW = 32
QSCALE = (DH ** -0.5) * math.log2(math.e)
NT = (((1,), (1,)), ((), ()))
F32 = jnp.float32
BF16 = jnp.bfloat16
U32 = jnp.uint32
TQ = 512
CK = 128
NQ = S // TQ
NC = S // CK
NU = H * NQ
TPC = TQ // CK

PR = 16
L = 128
LBS = (112, 112, 112, 112, 112, 128, 112, 128, 112, 112, 112, 112, 128, 112, 128)
NVT = (4, 4, 6, 6, 4, 6, 4, 4, 4, 4, 4, 6, 4, 6, 6, 6)
NMT = tuple(16 - n for n in NVT)
KV = 8 * sum(NVT)
NB = 8 * sum(NMT)
VOFF = [8 * sum(NVT[:t]) for t in range(NC + 1)]
MOFF = [8 * sum(NMT[:t]) for t in range(NC + 1)]
PW_A, PW_B = 27, 28
NE = 6
FAST0, FAST1 = 10, 80

GROUPS = [(bi * 6 + ab * 3, c) for bi in range(KV // 48)
          for (ab, c) in ((0, 0), (1, 3), (0, 1), (1, 0), (0, 2), (1, 1), (0, 3), (1, 2))]
NG = len(GROUPS)
POS = ([L] + [CK * (t + 1) + L for t in range(NC)]
       + [S + MOFF[t + 1] + LBS[t] for t in range(NC - 1)] + [S + NB + L])


def _group_windows():
    dur = [POS[i + 1] - POS[i] + 24 for i in range(2 * NC)]
    wins = []
    for gi in range(NG):
        if gi < NE:
            wins.append(-1)
            continue
        tgt = int((gi - NE) * sum(dur) * 0.9) // (NG - NE)
        cum, w = 0, 0
        while cum + dur[w] <= tgt:
            cum += dur[w]
            w += 1
        wins.append(w)
    for gi, (g0, _) in enumerate(GROUPS):
        for g in range(g0, g0 + 3):
            t = max(i for i in range(NC) if VOFF[i] <= 8 * g)
            assert wins[gi] <= NC + t
            assert wins[gi] + NC > t
    return wins


GWIN = _group_windows()


def _kernel(xa_hbm, wa_hbm, woa_hbm, xb_hbm, wqb_hbm, wkb_hbm, wvb_hbm, wob_hbm, o_hbm,
            xa_ref, wa_ref, woa_ref, xb_ref, wqb_ref, wob_ref, o_ref, isem, xsem, osem,
            wsm_scr, ka_scr, kb_scr, kbn_scr, qta, qtb, vta, vtb, ota, otb, pc, sv, kbc,
            zero_scr, wkb_ref, wvb_ref, flag):
    def mo(x, m):
        return x if isinstance(x, int) else pl.multiple_of(x, m)

    def cp(src, dst, i):
        return pltpu.make_async_copy(src, dst, isem.at[i])

    def xb_cp(r):
        rows = pl.ds(mo(r * TQ, TQ), TQ)
        return pltpu.make_async_copy(xb_hbm.at[0, rows, :], xb_ref.at[rows, :], xsem.at[r])

    c_wqb = cp(wqb_hbm, wqb_ref, 0)
    c_wkb = cp(wkb_hbm, wkb_ref, 1)
    c_wvb = cp(wvb_hbm, wvb_ref, 2)
    c_wa = cp(wa_hbm, wa_ref, 3)
    c_xa = cp(xa_hbm.at[0], xa_ref, 4)
    c_woa = cp(woa_hbm, woa_ref, 5)
    c_wob = cp(wob_hbm, wob_ref, 6)
    for c in (c_wkb, c_wvb, xb_cp(0), c_wqb):
        c.start()

    zero_scr[...] = jnp.zeros((8, 128), jnp.int32)
    rows24 = jax.lax.broadcasted_iota(jnp.int32, (HP, TQ), 0)
    vfill = jnp.where(rows24 == DH, 1.0, 0.0)

    def head_rows(x, h, fill):
        if DH * h + HP <= x.shape[0]:
            w = x[DH * h:DH * h + HP]
        else:
            w = jnp.concatenate([x[DH * h:], x[:DH * h + HP - x.shape[0]]], axis=0)
        return jnp.where(rows24 < DH, w, fill)

    def kload(ref, idx, r0, n):
        return pltpu.bitcast(ref[idx, pl.ds(r0 // 2, n // 2), :], BF16)

    def qproj(x, w, qt_scr, qi):
        q = (jnp.dot(x, w, preferred_element_type=F32) * QSCALE).astype(BF16)
        qt = q.T.astype(F32)
        for h in range(H):
            qt_scr[qi, h] = head_rows(qt, h, 0.0)

    c_wkb.wait()
    c_wvb.wait()
    wsm_scr[...] = jnp.concatenate(
        [wkb_ref[...].astype(F32), jnp.zeros((12, D), F32),
         wvb_ref[...].astype(F32), jnp.zeros((76, D), F32)], axis=0).astype(BF16)
    c_wqb.wait()
    for r in range(1, NQ):
        xb_cp(r).start()
    c_wa.start()
    c_xa.start()

    def bbody(r, _):
        r0 = pl.multiple_of(r * TQ, TQ)
        xb_cp(r).wait()
        x = xb_ref[pl.ds(r0, TQ), :]
        kv = jax.lax.dot_general(x, wsm_scr[...], NT, preferred_element_type=F32)
        lane = jax.lax.broadcasted_iota(jnp.int32, (TQ, 128), 1)
        kbn_scr[pl.ds(r0, TQ), :] = jnp.where(lane == HP, 1.0, kv).astype(BF16).astype(F32)
        vtb[0, :, pl.ds(r0, TQ)] = jnp.where(rows24 < DH, kv.T[KW:KW + HP, :], vfill)
        qproj(x, wqb_ref[...], qtb, r)
        return 0
    jax.lax.fori_loop(0, NQ, bbody, 0)

    c_woa.start()
    c_wob.start()
    c_wa.wait()
    c_xa.wait()
    lane32 = jax.lax.broadcasted_iota(jnp.int32, (TQ, KW), 1)

    def kvbody(r, _):
        r0 = pl.multiple_of(r * TQ, TQ)
        x = xa_ref[pl.ds(r0, TQ), :]
        k = jnp.dot(x, wa_ref[:, pl.ds(D, D)], preferred_element_type=F32)
        k = jnp.concatenate([k[t * CK + 8 * g:t * CK + 8 * g + 8] for t in range(TPC)
                             for g in range(15, -1, -1)], axis=0)
        fill = jnp.where(lane32 == HP, 1.0, 0.0)
        for h in range(H):
            w0 = DH * h
            if w0 + KW <= D:
                kw = k[:, w0:w0 + KW]
            else:
                kw = jnp.concatenate([k[:, w0:D], jnp.zeros((TQ, w0 + KW - D), F32)], axis=1)
            kh = jnp.where(lane32 < DH, kw, fill).astype(BF16)
            ka_scr[h, pl.ds(pl.multiple_of(r * (TQ // 2), TQ // 2), TQ // 2), :] = pltpu.bitcast(kh, U32)
        v = jnp.dot(x, wa_ref[:, pl.ds(2 * D, D)], preferred_element_type=F32).astype(BF16)
        vt = v.T.astype(F32)
        for h in range(H):
            vta[h, :, pl.ds(r0, TQ)] = head_rows(vt, h, vfill)
        return 0
    jax.lax.fori_loop(0, NQ, kvbody, 0)

    for r in range(NQ):
        qproj(xa_ref[pl.ds(r * TQ, TQ), :], wa_ref[:, pl.ds(0, D)], qta, r)
        for t in range(r * TPC, (r + 1) * TPC):
            km = jnp.concatenate([kbn_scr[pl.ds(t * CK + 8 * g, 8), :][:, :KW]
                                  for g in range(NMT[t] - 1, -1, -1)], axis=0).astype(BF16)
            kb_scr[0, pl.ds(MOFF[t] // 2, 4 * NMT[t]), :] = pltpu.bitcast(km, U32)
            kk = kbn_scr[pl.ds(t * CK + 8 * NMT[t], 8 * NVT[t]), :]
            for d in range(DH):
                kbc[d, pl.ds(VOFF[t], 8 * NVT[t]), :] = jnp.broadcast_to(kk[:, d:d + 1], (8 * NVT[t], 128))

    A = dict(qt=qta, vt=vta, ot=ota, k=ka_scr, a=True)
    B = dict(qt=qtb, vt=vtb, ot=otb, k=kb_scr, a=False)

    def uparams(u):
        if isinstance(u, int):
            return u // NQ, u % NQ
        return jax.lax.shift_right_logical(u, 2), jax.lax.bitwise_and(u, NQ - 1)

    def weights(br, u, negm):
        h, qi = uparams(u)
        w = jnp.concatenate([br['qt'][qi, h], negm], axis=0).astype(BF16)
        return w, (h if br['a'] else 0)

    def probe(br, u):
        w, kidx = weights(br, u, jnp.zeros((8, TQ), F32))
        s = jnp.dot(kload(br['k'], kidx, 0, PR), w, preferred_element_type=F32)
        m = jnp.max(s, axis=0, keepdims=True)
        nm = jnp.abs(m) * 2.0 ** -7 - m
        return jnp.broadcast_to(nm, (8, TQ)).astype(BF16).astype(F32)

    def qk(br, wk_, r0, n):
        w, kidx = wk_
        p = jnp.exp2(jnp.dot(kload(br['k'], kidx, r0, n), w, preferred_element_type=F32))
        return [p[t:t + 8] for t in range(0, n, 8)]

    def pv(br, u, t, groups, acc):
        h, _ = uparams(u)
        p = jnp.concatenate(groups[::-1], axis=0)
        v = br['vt'][h if br['a'] else 0, :, pl.ds(t * CK, CK)]
        o = jnp.dot(v, p, preferred_element_type=F32)
        return o if acc is None else o + acc

    def vpu_group(gi, u, nm, never, dep):
        h, qi = uparams(u)
        g0, jj = GROUPS[gi]
        init = nm[:, jj * 128:(jj + 1) * 128]
        if dep is not None and FAST0 <= gi < FAST1:
            acc = jnp.concatenate(
                [jnp.where(never, dep[8 * ((c + 1) % 3):8 * ((c + 1) % 3) + 8], init) for c in range(3)], axis=0)
        else:
            if dep is not None:
                init = jnp.where(never, jnp.maximum(jnp.maximum(dep[0:8], dep[8:16]), dep[16:24]), init)
            acc = jnp.concatenate([init] * 3, axis=0)
        for d in range(DH):
            acc = acc + kbc[d, pl.ds(g0 * 8, 24), :] * qtb[qi, h, pl.ds(d, 1), pl.ds(jj * 128, 128)]
        sv[pl.ds(g0 * 8, 24), pl.ds(jj * 128, 128)] = acc
        return acc

    def body(j, carry):
        nm_a, nm_b = carry
        jn = jnp.minimum(j + 1, NU - 1)
        never = zero_scr[...] != 0
        wts = {'A': weights(A, j, nm_a), 'B': weights(B, j, nm_b)}
        stream = [pc[pl.ds(t, 8), :] for t in range(0, L, 8)]
        acc = None
        dep = None
        for w in range(2 * NC):
            for (lo, hi, br, key) in ((0, S, A, 'A'), (S, S + NB, B, 'B'), (S + NB, S + NB + L, A, 'N')):
                x0, x1 = max(POS[w], lo), min(POS[w + 1], hi)
                if x0 < x1:
                    if key not in wts:
                        wts[key] = weights(A, jn, nm_a2)
                    out = qk(br, wts[key], x0 - lo, x1 - x0)
                    if key == 'N':
                        for i, g in enumerate(out):
                            pc[pl.ds(x0 - lo + 8 * i, 8), :] = g
                    else:
                        stream += out
            if w == PW_A:
                nm_a2 = probe(A, jn)
            if w == PW_B:
                nm_b2 = probe(B, jn)
            for gi in range(NG):
                if GWIN[gi] == w:
                    dep = vpu_group(gi, j, nm_b, never, dep)
            if w == 2 * NC - 1:
                for gi in range(NE):
                    dep = vpu_group(gi, jn, nm_b2, never, dep)
            if w < NC:
                acc = pv(A, j, w, stream[16 * w:16 * w + 16], acc)
            else:
                t = w - NC
                s0 = 16 * NC + MOFF[t] // 8
                vg = [jnp.exp2(sv[pl.ds(VOFF[t] + 8 * g, 8), :]) for g in range(NVT[t] - 1, -1, -1)]
                acc = pv(B, j, t, vg + stream[s0:s0 + NMT[t]], acc)
            if w % NC == NC - 1:
                h, qi = uparams(j)
                (ota if w < NC else otb)[qi, h] = acc
                acc = None
        return nm_a2, nm_b2

    nm_a0 = probe(A, 0)
    nm_b0 = probe(B, 0)
    for i, g in enumerate(qk(A, weights(A, 0, nm_a0), 0, L)):
        pc[pl.ds(8 * i, 8), :] = g
    for gi in range(NE):
        vpu_group(gi, 0, nm_b0, None, None)
    jax.lax.fori_loop(0, NU, body, (nm_a0, nm_b0))

    def slow(br):
        def unit(u, _):
            h, qi = uparams(u)
            w, kidx = weights(br, u, jnp.zeros((8, TQ), F32))

            def scores(t):
                if br['a']:
                    k = pltpu.bitcast(
                        ka_scr[kidx, pl.ds(pl.multiple_of(t * (CK // 2), CK // 2), CK // 2), :], BF16)
                    s = jnp.dot(k, w, preferred_element_type=F32)
                    return jnp.concatenate([s[8 * g:8 * g + 8] for g in range(15, -1, -1)], axis=0)
                k = kbn_scr[pl.ds(pl.multiple_of(t * CK, CK), CK), :][:, :KW].astype(BF16)
                return jnp.dot(k, w, preferred_element_type=F32)

            m = jax.lax.fori_loop(
                0, NC, lambda t, m: jnp.maximum(m, jnp.max(scores(t), axis=0, keepdims=True)),
                jnp.full((1, TQ), -jnp.inf, F32))

            def acc_tile(t, acc):
                p = jnp.exp2(scores(t) - m)
                v = br['vt'][kidx, :, pl.ds(pl.multiple_of(t * CK, CK), CK)]
                return acc + jnp.dot(v, p, preferred_element_type=F32)
            br['ot'][qi, h] = jax.lax.fori_loop(0, NC, acc_tile, jnp.zeros((HP, TQ), F32))
            return 0
        jax.lax.fori_loop(0, NU, unit, 0)

    c_woa.wait()
    c_wob.wait()

    def ocp(qi, i):
        rows = pl.ds(mo(qi * TQ, TQ), TQ)
        return pltpu.make_async_copy(o_ref.at[i, rows, :], o_hbm.at[0, rows, pl.ds(i * D, D)],
                                     osem.at[2 * qi + i])

    def obody(qi, chk):
        lmin, lmax, bad = chk
        for i, (ot, wo_ref) in enumerate(((ota, woa_ref), (otb, wob_ref))):
            parts = []
            for h in range(H):
                a = ot[qi, h]
                lmin = jnp.minimum(lmin, a[16:24])
                lmax = jnp.maximum(lmax, a[16:24])
                l = ot[qi, h, pl.ds(DH, 1), :]
                r = pl.reciprocal(l, approx=True)
                r = r * (2.0 - l * r)
                parts.append((a * r)[:DH])
            o = jnp.concatenate(parts, axis=0).T.astype(BF16)
            y = jnp.dot(o, wo_ref[...], preferred_element_type=F32)
            nonfinite = jnp.where(jnp.abs(y) < 2.0 ** 127, 0.0, 1.0)
            bad = jnp.maximum(bad, jnp.max(nonfinite.reshape(TQ // 8, 8, D), axis=0))
            o_ref[i, pl.ds(pl.multiple_of(qi * TQ, TQ), TQ), :] = y.astype(o_ref.dtype)
            ocp(qi, i).start()
        return lmin, lmax, bad

    flag[0] = 1

    def attempt(p, _):
        @pl.when(flag[0] != 0)
        def _():
            @pl.when(p == 1)
            def _():
                slow(A)
                slow(B)
            one = jnp.ones((8, TQ), F32)
            lmin, lmax, bad = jax.lax.fori_loop(0, NQ, obody, (one, one, jnp.zeros((8, D), F32)))
            lok = jnp.logical_and(lmin[DH - 16:DH - 15] > 0.5, lmax[DH - 16:DH - 15] < 2.0 ** 100)
            nbad = jnp.max(bad) + jnp.max(jnp.where(lok, 0.0, 1.0))
            flag[0] = jnp.where(nbad > 0.0, 1, 0)
            for qi in range(NQ):
                for i in range(2):
                    ocp(qi, i).wait()
        return 0
    jax.lax.fori_loop(0, 2, attempt, 0)


@jax.jit
def pallas_concat_heads__softmax_full_mha__grouped_kv_mqa__prompt_kernel(
    A_x: jax.Array,
    A_wqkv: jax.Array,
    A_wo: jax.Array,
    B_x: jax.Array,
    B_wq: jax.Array,
    B_wk: jax.Array,
    B_wv: jax.Array,
    B_wo: jax.Array,
):
    return pl.pallas_call(
        _kernel,
        in_specs=[pl.BlockSpec(memory_space=pl.ANY)] * 8,
        out_specs=pl.BlockSpec(memory_space=pl.ANY),
        out_shape=jax.ShapeDtypeStruct((1, S, 2 * D), BF16),
        scratch_shapes=[
            pltpu.VMEM((S, D), BF16),
            pltpu.VMEM((D, 3 * D), BF16),
            pltpu.VMEM((D, D), BF16),
            pltpu.VMEM((S, D), BF16),
            pltpu.VMEM((D, D), BF16),
            pltpu.VMEM((D, D), BF16),
            pltpu.VMEM((2, S, D), BF16),
            pltpu.SemaphoreType.DMA((7,)),
            pltpu.SemaphoreType.DMA((NQ,)),
            pltpu.SemaphoreType.DMA((2 * NQ,)),
            pltpu.VMEM((128, D), BF16),
            pltpu.VMEM((H, S // 2, KW), U32),
            pltpu.VMEM((1, S // 2, KW), U32),
            pltpu.VMEM((S, 128), F32),
            pltpu.VMEM((NQ, H, HP, TQ), F32),
            pltpu.VMEM((NQ, H, HP, TQ), F32),
            pltpu.VMEM((H, HP, S), F32),
            pltpu.VMEM((1, HP, S), F32),
            pltpu.VMEM((NQ, H, HP, TQ), F32),
            pltpu.VMEM((NQ, H, HP, TQ), F32),
            pltpu.VMEM((L, TQ), F32),
            pltpu.VMEM((768, TQ), F32),
            pltpu.VMEM((DH, 768, 128), F32),
            pltpu.VMEM((8, 128), jnp.int32),
            pltpu.VMEM((DH, D), BF16),
            pltpu.VMEM((DH, D), BF16),
            pltpu.SMEM((1,), jnp.int32),
        ],
        compiler_params=pltpu.CompilerParams(vmem_limit_bytes=110 * 1024 * 1024),
    )(A_x, A_wqkv, A_wo, B_x, B_wq, B_wk.T, B_wv.T, B_wo)
```

```python
import math

import jax
import jax.numpy as jnp
import jax.experimental.pallas as pl
import jax.experimental.pallas.tpu as pltpu

S = 2048
D = 640
H = 32
DH = 20
HP = 24
KW = 32
QSCALE = (DH ** -0.5) * math.log2(math.e)
NT = (((1,), (1,)), ((), ()))
F32 = jnp.float32
BF16 = jnp.bfloat16
U32 = jnp.uint32
TQ = 512
CK = 128
NQ = S // TQ
NC = S // CK
NU = H * NQ
TPC = TQ // CK

L = 128
LAS = (128, 144, 144, 144, 144, 128, 144, 128, 128, 144, 128, 128, 128, 128, 128, 128)
LBS = (112, 128, 112, 112, 112, 128, 112, 128, 112, 128, 112, 96, 112, 112, 128)
NVT = (6, 6, 6, 6, 4, 4, 4, 6, 4, 4, 4, 6, 4, 6, 6, 6)
NMT = tuple(16 - n for n in NVT)
NB = 8 * sum(NMT)
VOFF = [8 * sum(NVT[:t]) for t in range(NC + 1)]
MOFF = [8 * sum(NMT[:t]) for t in range(NC + 1)]
WID = [4] * 4 + [3] * 22
SOFF = [sum(WID[:i]) for i in range(len(WID) + 1)]
assert SOFF[-1] == sum(NVT)
GROUPS = [(SOFF[2 * bi + ab], WID[2 * bi + ab], c) for bi in range(len(WID) // 2)
          for (ab, c) in ((0, 0), (1, 3), (0, 1), (1, 0), (0, 2), (1, 1), (0, 3), (1, 2))]
NG = len(GROUPS)
NE = 2
RELW = 30
FAST0 = 18
POS = ([L] + [CK * (t + 1) + LAS[t] for t in range(NC)]
       + [S + MOFF[t + 1] + LBS[t] for t in range(NC - 1)] + [S + NB + L])


def _group_windows():
    dur = [POS[i + 1] - POS[i] + 24 for i in range(2 * NC)]
    wins = []
    for gi in range(NG):
        if gi < NE:
            wins.append(-1)
            continue
        tgt = int((gi - NE) * sum(dur) * 0.9) // (NG - NE)
        cum, w = 0, 0
        while cum + dur[w] <= tgt:
            cum += dur[w]
            w += 1
        wins.append(w)
    for gi, (g0, wd, _) in enumerate(GROUPS):
        for g in range(g0, g0 + wd):
            t = max(i for i in range(NC) if VOFF[i] <= 8 * g)
            assert wins[gi] <= NC + t
            assert wins[gi] + NC > t
    return wins


GWIN = _group_windows()


def _kernel(xa_hbm, wa_hbm, woa_hbm, xb_hbm, wqb_hbm, wkb_hbm, wvb_hbm, wob_hbm, o_hbm,
            xa_ref, wa_ref, woa_ref, xb_ref, wqb_ref, wob_ref, o_ref, isem, xsem, osem,
            wsm_scr, ka_scr, kb_scr, kbn_scr, qta, qtb, vta, vtb, ota, otb, pc, sv, kbc,
            zero_scr, wkb_ref, wvb_ref, flag):
    def mo(x, m):
        return x if isinstance(x, int) else pl.multiple_of(x, m)

    def cp(src, dst, i):
        return pltpu.make_async_copy(src, dst, isem.at[i])

    def xb_cp(r):
        rows = pl.ds(mo(r * TQ, TQ), TQ)
        return pltpu.make_async_copy(xb_hbm.at[0, rows, :], xb_ref.at[rows, :], xsem.at[r])

    c_wqb = cp(wqb_hbm, wqb_ref, 0)
    c_wkb = cp(wkb_hbm, wkb_ref, 1)
    c_wvb = cp(wvb_hbm, wvb_ref, 2)
    c_wa = cp(wa_hbm, wa_ref, 3)
    c_xa = cp(xa_hbm.at[0], xa_ref, 4)
    c_woa = cp(woa_hbm, woa_ref, 5)
    c_wob = cp(wob_hbm, wob_ref, 6)
    for c in (c_wkb, c_wvb, xb_cp(0), c_wqb):
        c.start()

    zero_scr[...] = jnp.zeros((8, 128), jnp.int32)
    rows24 = jax.lax.broadcasted_iota(jnp.int32, (HP, TQ), 0)
    rows8 = jax.lax.broadcasted_iota(jnp.int32, (8, TQ), 0)
    vfill = jnp.where(rows24 == DH, 1.0, 0.0)

    def head_window(x, h):
        if DH * h + HP <= x.shape[0]:
            return x[DH * h:DH * h + HP]
        return jnp.concatenate([x[DH * h:], x[:DH * h + HP - x.shape[0]]], axis=0)

    def head_rows(x, h, fill):
        return jnp.where(rows24 < DH, head_window(x, h), fill)

    def kload(ref, idx, r0, n):
        return pltpu.bitcast(ref[idx, pl.ds(r0 // 2, n // 2), :], BF16)

    def qproj(x, w, qt_scr, qi, kcol):
        q = (jnp.dot(x, w, preferred_element_type=F32) * QSCALE).astype(BF16)
        qt = q.T.astype(F32)
        for h in range(H):
            b = head_rows(qt, h, 0.0)
            m = jnp.sum(b * jnp.concatenate([kcol(h)] * (TQ // 128), axis=1), axis=0, keepdims=True)
            rem = jnp.broadcast_to(-m, (8, TQ))
            top = b[16:]
            for i in range(3):
                top = jnp.where(rows8 == DH - 16 + i, rem, top)
                if i < 2:
                    rem = rem - rem.astype(BF16).astype(F32)
            qt_scr[qi, h] = jnp.concatenate([b[:16], top], axis=0)

    c_wkb.wait()
    c_wvb.wait()
    wsm_scr[...] = jnp.concatenate(
        [wkb_ref[...].astype(F32), jnp.zeros((12, D), F32),
         wvb_ref[...].astype(F32), jnp.zeros((76, D), F32)], axis=0).astype(BF16)
    c_wqb.wait()
    for r in range(1, NQ):
        xb_cp(r).start()
    c_wa.start()
    c_xa.start()

    def bbody(r, kc):
        r0 = pl.multiple_of(r * TQ, TQ)
        xb_cp(r).wait()
        x = xb_ref[pl.ds(r0, TQ), :]
        kv = jax.lax.dot_general(x, wsm_scr[...], NT, preferred_element_type=F32)
        lane = jax.lax.broadcasted_iota(jnp.int32, (TQ, 128), 1)
        kv = kv.astype(BF16).astype(F32)
        kbn_scr[pl.ds(r0, TQ), :] = jnp.where(jnp.logical_and(lane >= DH, lane < HP), 1.0, kv)
        kvt = kv.T
        vtb[0, :, pl.ds(r0, TQ)] = jnp.where(rows24 < DH, kvt[KW:KW + HP, :], vfill)
        kc = jnp.where(r == 0, jnp.broadcast_to(jnp.mean(kvt[:HP, :CK], axis=1, keepdims=True), (HP, 128)), kc)
        qproj(x, wqb_ref[...], qtb, r, lambda h: kc)
        return kc
    kcb = jax.lax.fori_loop(0, NQ, bbody, jnp.zeros((HP, 128), F32))

    c_woa.start()
    c_wob.start()
    c_wa.wait()
    c_xa.wait()
    lane32 = jax.lax.broadcasted_iota(jnp.int32, (TQ, KW), 1)

    def kvbody(r, kmean):
        r0 = pl.multiple_of(r * TQ, TQ)
        x = xa_ref[pl.ds(r0, TQ), :]
        k = jnp.dot(x, wa_ref[:, pl.ds(D, D)], preferred_element_type=F32)
        kmean = jnp.where(r == 0, jnp.mean(k[:CK], axis=0, keepdims=True), kmean)
        k = jnp.concatenate([k[t * CK + 8 * g:t * CK + 8 * g + 8] for t in range(TPC)
                             for g in range(15, -1, -1)], axis=0)
        for h in range(H):
            w0 = DH * h
            if w0 + KW <= D:
                kw = k[:, w0:w0 + KW]
            else:
                kw = jnp.concatenate([k[:, w0:D], jnp.zeros((TQ, w0 + KW - D), F32)], axis=1)
            ka_scr[h, pl.ds(pl.multiple_of(r * (TQ // 2), TQ // 2), TQ // 2), :] = pltpu.bitcast(
                jnp.where(lane32 >= DH, 1.0, kw).astype(BF16), U32)
        v = jnp.dot(x, wa_ref[:, pl.ds(2 * D, D)], preferred_element_type=F32).astype(BF16)
        vt = v.T.astype(F32)
        for h in range(H):
            vta[h, :, pl.ds(r0, TQ)] = head_rows(vt, h, vfill)
        return kmean
    kmean = jax.lax.fori_loop(0, NQ, kvbody, jnp.zeros((1, D), F32))
    kmean_b = jnp.concatenate([kcb, jnp.zeros((128 - HP, 128), F32)], axis=0).T[:1]
    kca = jnp.broadcast_to(kmean, (128, D)).T

    for r in range(NQ):
        qproj(xa_ref[pl.ds(r * TQ, TQ), :], wa_ref[:, pl.ds(0, D)], qta, r, lambda h: head_window(kca, h))
        for t in range(r * TPC, (r + 1) * TPC):
            kt = kbn_scr[pl.ds(t * CK, CK), :]
            km = jnp.concatenate([kt[8 * g:8 * g + 8, :KW] for g in range(NMT[t] - 1, -1, -1)],
                                 axis=0).astype(BF16)
            kb_scr[0, pl.ds(MOFF[t] // 2, 4 * NMT[t]), :] = pltpu.bitcast(km, U32)
            kk = kt[8 * NMT[t]:] - kmean_b
            for d in range(DH):
                kbc[d, pl.ds(VOFF[t], 8 * NVT[t]), :] = jnp.broadcast_to(kk[:, d:d + 1], (8 * NVT[t], 128))

    A = dict(qt=qta, vt=vta, ot=ota, k=ka_scr, a=True)
    B = dict(qt=qtb, vt=vtb, ot=otb, k=kb_scr, a=False)

    def uparams(u):
        if isinstance(u, int):
            return u // NQ, u % NQ
        return jax.lax.shift_right_logical(u, 2), jax.lax.bitwise_and(u, NQ - 1)

    def weights(br, u):
        h, qi = uparams(u)
        w = jnp.concatenate([br['qt'][qi, h], jnp.zeros((KW - HP, TQ), F32)], axis=0).astype(BF16)
        return w, (h if br['a'] else 0)

    def qk(br, wk_, r0, n):
        w, kidx = wk_
        p = jnp.exp2(jnp.dot(kload(br['k'], kidx, r0, n), w, preferred_element_type=F32))
        return [p[t:t + 8] for t in range(0, n, 8)]

    def pv(br, u, t, groups, acc):
        h, _ = uparams(u)
        p = jnp.concatenate(groups[::-1], axis=0)
        v = br['vt'][h if br['a'] else 0, :, pl.ds(t * CK, CK)]
        o = jnp.dot(v, p, preferred_element_type=F32)
        return o if acc is None else o + acc

    def vpu_group(gi, u, never, dep, tok=None):
        h, qi = uparams(u)
        g0, wd, jj = GROUPS[gi]
        cols = pl.ds(jj * 128, 128)
        rows = pl.ds(g0 * 8, wd * 8)
        if dep is not None and gi >= FAST0:
            acc = kbc[0, rows, :] * qtb[qi, h, pl.ds(0, 1), cols]
            acc = jnp.concatenate(
                [jnp.where(never, dep[8 * ((c + 1) % wd):8 * ((c + 1) % wd) + 8], acc[8 * c:8 * c + 8])
                 for c in range(wd)], axis=0)
        else:
            q0 = jnp.broadcast_to(qtb[qi, h, pl.ds(0, 1), cols], (8, 128))
            if dep is not None:
                parts = [dep[8 * c:8 * c + 8] for c in range(dep.shape[0] // 8)]
                if tok is not None:
                    parts = [tok] + parts
                while len(parts) > 1:
                    parts = [jnp.maximum(parts[i], parts[i + 1]) if i + 1 < len(parts) else parts[i]
                             for i in range(0, len(parts), 2)]
                q0 = jnp.where(never, parts[0], q0)
            acc = kbc[0, rows, :] * jnp.concatenate([q0] * wd, axis=0)
        for d in range(1, DH):
            acc = acc + kbc[d, rows, :] * qtb[qi, h, pl.ds(d, 1), cols]
        sv[rows, cols] = acc
        return acc

    def body(j, carry):
        jn = jnp.minimum(j + 1, NU - 1)
        never = zero_scr[...] != 0
        wts = {'A': weights(A, j), 'B': weights(B, j)}
        stream = [pc[pl.ds(t, 8), :] for t in range(0, L, 8)]
        acc = None
        dep = None
        tok = None
        for w in range(2 * NC):
            for (lo, hi, br, key) in ((0, S, A, 'A'), (S, S + NB, B, 'B'), (S + NB, S + NB + L, A, 'N')):
                x0, x1 = max(POS[w], lo), min(POS[w + 1], hi)
                if x0 < x1:
                    if key not in wts:
                        wts[key] = weights(A, jn)
                    out = qk(br, wts[key], x0 - lo, x1 - x0)
                    if w == RELW:
                        tok = out[-1][:, :128]
                    if key == 'N':
                        for i, g in enumerate(out):
                            pc[pl.ds(x0 - lo + 8 * i, 8), :] = g
                    else:
                        stream += out
            for gi in range(NG):
                if GWIN[gi] == w:
                    dep = vpu_group(gi, j, never, dep)
            if w == 2 * NC - 1:
                for gi in range(NE):
                    dep = vpu_group(gi, jn, never, dep, tok if gi == 0 else None)
            if w < NC:
                acc = pv(A, j, w, stream[16 * w:16 * w + 16], acc)
            else:
                t = w - NC
                s0 = 16 * NC + MOFF[t] // 8
                vg = [jnp.exp2(sv[pl.ds(VOFF[t] + 8 * g, 8), :]) for g in range(NVT[t] - 1, -1, -1)]
                acc = pv(B, j, t, vg + stream[s0:s0 + NMT[t]], acc)
            if w % NC == NC - 1:
                h, qi = uparams(j)
                (ota if w < NC else otb)[qi, h] = acc
                acc = None
        return carry

    for i, g in enumerate(qk(A, weights(A, 0), 0, L)):
        pc[pl.ds(8 * i, 8), :] = g
    for gi in range(NE):
        vpu_group(gi, 0, None, None)
    jax.lax.fori_loop(0, NU, body, 0)

    def slow(br):
        def unit(u, _):
            h, qi = uparams(u)
            w, kidx = weights(br, u)

            def scores(t):
                if br['a']:
                    k = pltpu.bitcast(
                        ka_scr[kidx, pl.ds(pl.multiple_of(t * (CK // 2), CK // 2), CK // 2), :], BF16)
                    s = jnp.dot(k, w, preferred_element_type=F32)
                    return jnp.concatenate([s[8 * g:8 * g + 8] for g in range(15, -1, -1)], axis=0)
                k = kbn_scr[pl.ds(pl.multiple_of(t * CK, CK), CK), :][:, :KW].astype(BF16)
                return jnp.dot(k, w, preferred_element_type=F32)

            m = jax.lax.fori_loop(
                0, NC, lambda t, m: jnp.maximum(m, jnp.max(scores(t), axis=0, keepdims=True)),
                jnp.full((1, TQ), -jnp.inf, F32))

            def acc_tile(t, acc):
                p = jnp.exp2(scores(t) - m)
                v = br['vt'][kidx, :, pl.ds(pl.multiple_of(t * CK, CK), CK)]
                return acc + jnp.dot(v, p, preferred_element_type=F32)
            br['ot'][qi, h] = jax.lax.fori_loop(0, NC, acc_tile, jnp.zeros((HP, TQ), F32))
            return 0
        jax.lax.fori_loop(0, NU, unit, 0)

    c_woa.wait()
    c_wob.wait()

    def ocp(qi, i):
        rows = pl.ds(mo(qi * TQ, TQ), TQ)
        return pltpu.make_async_copy(o_ref.at[i, rows, :], o_hbm.at[0, rows, pl.ds(i * D, D)],
                                     osem.at[2 * qi + i])

    def obody(qi, chk):
        lmin, lmax, bad = chk
        for i, (ot, wo_ref) in enumerate(((ota, woa_ref), (otb, wob_ref))):
            parts = []
            for h in range(H):
                a = ot[qi, h]
                lmin = jnp.minimum(lmin, a[16:24])
                lmax = jnp.maximum(lmax, a[16:24])
                l = ot[qi, h, pl.ds(DH, 1), :]
                r = pl.reciprocal(l, approx=True)
                r = r * (2.0 - l * r)
                parts.append((a * r)[:DH])
            o = jnp.concatenate(parts, axis=0).T.astype(BF16)
            y = jnp.dot(o, wo_ref[...], preferred_element_type=F32)
            nonfinite = jnp.where(jnp.abs(y) < 2.0 ** 127, 0.0, 1.0)
            bad = jnp.maximum(bad, jnp.max(nonfinite.reshape(TQ // 8, 8, D), axis=0))
            o_ref[i, pl.ds(pl.multiple_of(qi * TQ, TQ), TQ), :] = y.astype(o_ref.dtype)
            ocp(qi, i).start()
        return lmin, lmax, bad

    flag[0] = 1

    def attempt(p, _):
        @pl.when(flag[0] != 0)
        def _():
            @pl.when(p == 1)
            def _():
                slow(A)
                slow(B)
            one = jnp.ones((8, TQ), F32)
            lmin, lmax, bad = jax.lax.fori_loop(0, NQ, obody, (one, one, jnp.zeros((8, D), F32)))
            lok = jnp.logical_and(lmin[DH - 16:DH - 15] >= 1.0, lmax[DH - 16:DH - 15] < 2.0 ** 100)
            nbad = jnp.max(bad) + jnp.max(jnp.where(lok, 0.0, 1.0))
            flag[0] = jnp.where(nbad > 0.0, 1, 0)
            for qi in range(NQ):
                for i in range(2):
                    ocp(qi, i).wait()
        return 0
    jax.lax.fori_loop(0, 2, attempt, 0)


@jax.jit
def pallas_concat_heads__softmax_full_mha__grouped_kv_mqa__prompt_kernel(
    A_x: jax.Array,
    A_wqkv: jax.Array,
    A_wo: jax.Array,
    B_x: jax.Array,
    B_wq: jax.Array,
    B_wk: jax.Array,
    B_wv: jax.Array,
    B_wo: jax.Array,
):
    return pl.pallas_call(
        _kernel,
        in_specs=[pl.BlockSpec(memory_space=pl.ANY)] * 8,
        out_specs=pl.BlockSpec(memory_space=pl.ANY),
        out_shape=jax.ShapeDtypeStruct((1, S, 2 * D), BF16),
        scratch_shapes=[
            pltpu.VMEM((S, D), BF16),
            pltpu.VMEM((D, 3 * D), BF16),
            pltpu.VMEM((D, D), BF16),
            pltpu.VMEM((S, D), BF16),
            pltpu.VMEM((D, D), BF16),
            pltpu.VMEM((D, D), BF16),
            pltpu.VMEM((2, S, D), BF16),
            pltpu.SemaphoreType.DMA((7,)),
            pltpu.SemaphoreType.DMA((NQ,)),
            pltpu.SemaphoreType.DMA((2 * NQ,)),
            pltpu.VMEM((128, D), BF16),
            pltpu.VMEM((H, S // 2, KW), U32),
            pltpu.VMEM((1, S // 2, KW), U32),
            pltpu.VMEM((S, 128), F32),
            pltpu.VMEM((NQ, H, HP, TQ), F32),
            pltpu.VMEM((NQ, H, HP, TQ), F32),
            pltpu.VMEM((H, HP, S), F32),
            pltpu.VMEM((1, HP, S), F32),
            pltpu.VMEM((NQ, H, HP, TQ), F32),
            pltpu.VMEM((NQ, H, HP, TQ), F32),
            pltpu.VMEM((L, TQ), F32),
            pltpu.VMEM((768, TQ), F32),
            pltpu.VMEM((DH, 768, 128), F32),
            pltpu.VMEM((8, 128), jnp.int32),
            pltpu.VMEM((DH, D), BF16),
            pltpu.VMEM((DH, D), BF16),
            pltpu.SMEM((1,), jnp.int32),
        ],
        compiler_params=pltpu.CompilerParams(vmem_limit_bytes=110 * 1024 * 1024),
    )(A_x, A_wqkv, A_wo, B_x, B_wq, B_wk.T, B_wv.T, B_wo)
```

```python
import math

import jax
import jax.numpy as jnp
import jax.experimental.pallas as pl
import jax.experimental.pallas.tpu as pltpu

S = 2048
D = 640
H = 32
DH = 20
HP = 24
KW = 32
QSCALE = (DH ** -0.5) * math.log2(math.e)
NT = (((1,), (1,)), ((), ()))
F32 = jnp.float32
BF16 = jnp.bfloat16
U32 = jnp.uint32
TQ = 512
CK = 128
NQ = S // TQ
NC = S // CK
NU = H * NQ
TPC = TQ // CK

L = 128
LAS = (128, 144, 144, 144, 144, 128, 144, 128, 128, 144, 128, 128, 128, 128, 128, 128)
LBS = (112, 128, 112, 112, 112, 128, 112, 128, 112, 128, 112, 96, 112, 112, 128)
NVT = (6, 6, 6, 6, 4, 4, 4, 6, 4, 4, 4, 6, 4, 6, 6, 6)
NMT = tuple(16 - n for n in NVT)
NB = 8 * sum(NMT)
VOFF = [8 * sum(NVT[:t]) for t in range(NC + 1)]
MOFF = [8 * sum(NMT[:t]) for t in range(NC + 1)]
WID = [4] * 4 + [3] * 22
SOFF = [sum(WID[:i]) for i in range(len(WID) + 1)]
assert SOFF[-1] == sum(NVT)
GROUPS = [(SOFF[2 * bi + ab], WID[2 * bi + ab], c) for bi in range(len(WID) // 2)
          for (ab, c) in ((0, 0), (1, 3), (0, 1), (1, 0), (0, 2), (1, 1), (0, 3), (1, 2))]
NG = len(GROUPS)
NE = 2
RELW = 30
FAST0 = 18
POS = ([L] + [CK * (t + 1) + LAS[t] for t in range(NC)]
       + [S + MOFF[t + 1] + LBS[t] for t in range(NC - 1)] + [S + NB + L])


def _group_windows():
    dur = [POS[i + 1] - POS[i] + 24 for i in range(2 * NC)]
    wins = []
    for gi in range(NG):
        if gi < NE:
            wins.append(-1)
            continue
        tgt = int((gi - NE) * sum(dur) * 0.9) // (NG - NE)
        cum, w = 0, 0
        while cum + dur[w] <= tgt:
            cum += dur[w]
            w += 1
        wins.append(w)
    for gi, (g0, wd, _) in enumerate(GROUPS):
        for g in range(g0, g0 + wd):
            t = max(i for i in range(NC) if VOFF[i] <= 8 * g)
            assert wins[gi] <= NC + t
            assert wins[gi] + NC > t
    return wins


GWIN = _group_windows()


def _kernel(xa_hbm, wa_hbm, woa_hbm, xb_hbm, wqb_hbm, wkb_hbm, wvb_hbm, wob_hbm, o_hbm,
            xa_ref, wa_ref, woa_ref, xb_ref, wqb_ref, wob_ref, o_ref, isem, xsem, osem,
            wsm_scr, ka_scr, kb_scr, kbn_scr, qta, qtb, vta, vtb, ota, otb, pc, sv, kbc,
            zero_scr, wkb_ref, wvb_ref, flag):
    def mo(x, m):
        return x if isinstance(x, int) else pl.multiple_of(x, m)

    def cp(src, dst, i):
        return pltpu.make_async_copy(src, dst, isem.at[i])

    def xb_cp(r):
        rows = pl.ds(mo(r * TQ, TQ), TQ)
        return pltpu.make_async_copy(xb_hbm.at[0, rows, :], xb_ref.at[rows, :], xsem.at[r])

    c_wqb = cp(wqb_hbm, wqb_ref, 0)
    c_wkb = cp(wkb_hbm, wkb_ref, 1)
    c_wvb = cp(wvb_hbm, wvb_ref, 2)
    c_wa = cp(wa_hbm, wa_ref, 3)
    c_xa = cp(xa_hbm.at[0], xa_ref, 4)
    c_woa = cp(woa_hbm, woa_ref, 5)
    c_wob = cp(wob_hbm, wob_ref, 6)
    for c in (c_wkb, c_wvb, xb_cp(0), c_wqb):
        c.start()

    zero_scr[...] = jnp.zeros((8, 128), jnp.int32)
    rows24 = jax.lax.broadcasted_iota(jnp.int32, (HP, TQ), 0)
    rows8 = jax.lax.broadcasted_iota(jnp.int32, (8, TQ), 0)
    vfill = jnp.where(rows24 == DH, 1.0, 0.0)

    def head_window(x, h):
        if DH * h + HP <= x.shape[0]:
            return x[DH * h:DH * h + HP]
        return jnp.concatenate([x[DH * h:], x[:DH * h + HP - x.shape[0]]], axis=0)

    def head_rows(x, h, fill):
        return jnp.where(rows24 < DH, head_window(x, h), fill)

    def kload(ref, idx, r0, n):
        return pltpu.bitcast(ref[idx, pl.ds(r0 // 2, n // 2), :], BF16)

    def qproj(x, w, qt_scr, qi, kcol):
        q = (jnp.dot(x, w, preferred_element_type=F32) * QSCALE).astype(BF16)
        qt = q.T.astype(F32)
        for h in range(H):
            b = head_rows(qt, h, 0.0)
            m = jnp.sum(b * jnp.concatenate([kcol(h)] * (TQ // 128), axis=1), axis=0, keepdims=True)
            rem = jnp.broadcast_to(-m, (8, TQ))
            top = b[16:]
            for i in range(3):
                top = jnp.where(rows8 == DH - 16 + i, rem, top)
                if i < 2:
                    rem = rem - rem.astype(BF16).astype(F32)
            qt_scr[qi, h] = jnp.concatenate([b[:16], top], axis=0)

    c_wkb.wait()
    c_wvb.wait()
    wsm_scr[...] = jnp.concatenate(
        [wkb_ref[...].astype(F32), jnp.zeros((12, D), F32),
         wvb_ref[...].astype(F32), jnp.zeros((76, D), F32)], axis=0).astype(BF16)
    c_wqb.wait()
    for r in range(1, NQ):
        xb_cp(r).start()
    c_wa.start()
    c_xa.start()

    def bbody(r, kc):
        r0 = pl.multiple_of(r * TQ, TQ)
        xb_cp(r).wait()
        x = xb_ref[pl.ds(r0, TQ), :]
        kv = jax.lax.dot_general(x, wsm_scr[...], NT, preferred_element_type=F32)
        lane = jax.lax.broadcasted_iota(jnp.int32, (TQ, 128), 1)
        kv = kv.astype(BF16).astype(F32)
        kbn_scr[pl.ds(r0, TQ), :] = jnp.where(jnp.logical_and(lane >= DH, lane < HP), 1.0, kv)
        kvt = kv.T
        vtb[0, :, pl.ds(r0, TQ)] = jnp.where(rows24 < DH, kvt[KW:KW + HP, :], vfill)
        kc = jnp.where(r == 0, jnp.broadcast_to(jnp.mean(kvt[:HP, :CK], axis=1, keepdims=True), (HP, 128)), kc)
        qproj(x, wqb_ref[...], qtb, r, lambda h: kc)
        return kc
    kcb = jax.lax.fori_loop(0, NQ, bbody, jnp.zeros((HP, 128), F32))

    c_woa.start()
    c_wob.start()
    c_wa.wait()
    c_xa.wait()
    lane32 = jax.lax.broadcasted_iota(jnp.int32, (TQ, KW), 1)

    for r in range(NQ):
        x = xa_ref[pl.ds(r * TQ, TQ), :]
        k = jnp.dot(x, wa_ref[:, pl.ds(D, D)], preferred_element_type=F32)
        if r == 0:
            kmean = jnp.mean(k[:CK], axis=0, keepdims=True)
        k = jnp.concatenate([k[t * CK + 8 * g:t * CK + 8 * g + 8] for t in range(TPC)
                             for g in range(15, -1, -1)], axis=0)
        for h in range(H):
            w0 = DH * h
            if w0 + KW <= D:
                kw = k[:, w0:w0 + KW]
            else:
                kw = jnp.concatenate([k[:, w0:D], jnp.zeros((TQ, w0 + KW - D), F32)], axis=1)
            ka_scr[h, pl.ds(r * (TQ // 2), TQ // 2), :] = pltpu.bitcast(
                jnp.where(lane32 >= DH, 1.0, kw).astype(BF16), U32)
        v = jnp.dot(x, wa_ref[:, pl.ds(2 * D, D)], preferred_element_type=F32).astype(BF16)
        vt = v.T.astype(F32)
        for h in range(H):
            vta[h, :, pl.ds(r * TQ, TQ)] = head_rows(vt, h, vfill)
    kmean_b = jnp.concatenate([kcb, jnp.zeros((128 - HP, 128), F32)], axis=0).T[:1]
    kca = jnp.broadcast_to(kmean, (128, D)).T

    for r in range(NQ):
        qproj(xa_ref[pl.ds(r * TQ, TQ), :], wa_ref[:, pl.ds(0, D)], qta, r, lambda h: head_window(kca, h))
        for t in range(r * TPC, (r + 1) * TPC):
            kt = kbn_scr[pl.ds(t * CK, CK), :]
            km = jnp.concatenate([kt[8 * g:8 * g + 8, :KW] for g in range(NMT[t] - 1, -1, -1)],
                                 axis=0).astype(BF16)
            kb_scr[0, pl.ds(MOFF[t] // 2, 4 * NMT[t]), :] = pltpu.bitcast(km, U32)
            kk = kt[8 * NMT[t]:] - kmean_b
            for d in range(DH):
                kbc[d, pl.ds(VOFF[t], 8 * NVT[t]), :] = jnp.broadcast_to(kk[:, d:d + 1], (8 * NVT[t], 128))

    A = dict(qt=qta, vt=vta, ot=ota, k=ka_scr, a=True)
    B = dict(qt=qtb, vt=vtb, ot=otb, k=kb_scr, a=False)

    def uparams(u):
        if isinstance(u, int):
            return u // NQ, u % NQ
        return jax.lax.shift_right_logical(u, 2), jax.lax.bitwise_and(u, NQ - 1)

    def weights(br, u):
        h, qi = uparams(u)
        w = jnp.concatenate([br['qt'][qi, h], jnp.zeros((KW - HP, TQ), F32)], axis=0).astype(BF16)
        return w, (h if br['a'] else 0)

    def qk(br, wk_, r0, n):
        w, kidx = wk_
        p = jnp.exp2(jnp.dot(kload(br['k'], kidx, r0, n), w, preferred_element_type=F32))
        return [p[t:t + 8] for t in range(0, n, 8)]

    def pv(br, u, t, groups, acc):
        h, _ = uparams(u)
        p = jnp.concatenate(groups[::-1], axis=0)
        v = br['vt'][h if br['a'] else 0, :, pl.ds(t * CK, CK)]
        o = jnp.dot(v, p, preferred_element_type=F32)
        return o if acc is None else o + acc

    def vpu_group(gi, u, never, dep, tok=None):
        h, qi = uparams(u)
        g0, wd, jj = GROUPS[gi]
        cols = pl.ds(jj * 128, 128)
        rows = pl.ds(g0 * 8, wd * 8)
        if dep is not None and gi >= FAST0:
            acc = kbc[0, rows, :] * qtb[qi, h, pl.ds(0, 1), cols]
            acc = jnp.concatenate(
                [jnp.where(never, dep[8 * ((c + 1) % wd):8 * ((c + 1) % wd) + 8], acc[8 * c:8 * c + 8])
                 for c in range(wd)], axis=0)
        else:
            q0 = jnp.broadcast_to(qtb[qi, h, pl.ds(0, 1), cols], (8, 128))
            if dep is not None:
                parts = [dep[8 * c:8 * c + 8] for c in range(dep.shape[0] // 8)]
                if tok is not None:
                    parts = [tok] + parts
                while len(parts) > 1:
                    parts = [jnp.maximum(parts[i], parts[i + 1]) if i + 1 < len(parts) else parts[i]
                             for i in range(0, len(parts), 2)]
                q0 = jnp.where(never, parts[0], q0)
            acc = kbc[0, rows, :] * jnp.concatenate([q0] * wd, axis=0)
        for d in range(1, DH):
            acc = acc + kbc[d, rows, :] * qtb[qi, h, pl.ds(d, 1), cols]
        sv[rows, cols] = acc
        return acc

    def body(j, carry):
        jn = jnp.minimum(j + 1, NU - 1)
        never = zero_scr[...] != 0
        wts = {'A': weights(A, j), 'B': weights(B, j)}
        stream = [pc[pl.ds(t, 8), :] for t in range(0, L, 8)]
        acc = None
        dep = None
        tok = None
        for w in range(2 * NC):
            for (lo, hi, br, key) in ((0, S, A, 'A'), (S, S + NB, B, 'B'), (S + NB, S + NB + L, A, 'N')):
                x0, x1 = max(POS[w], lo), min(POS[w + 1], hi)
                if x0 < x1:
                    if key not in wts:
                        wts[key] = weights(A, jn)
                    out = qk(br, wts[key], x0 - lo, x1 - x0)
                    if w == RELW:
                        tok = out[-1][:, :128]
                    if key == 'N':
                        for i, g in enumerate(out):
                            pc[pl.ds(x0 - lo + 8 * i, 8), :] = g
                    else:
                        stream += out
            for gi in range(NG):
                if GWIN[gi] == w:
                    dep = vpu_group(gi, j, never, dep)
            if w == 2 * NC - 1:
                for gi in range(NE):
                    dep = vpu_group(gi, jn, never, dep, tok if gi == 0 else None)
            if w < NC:
                acc = pv(A, j, w, stream[16 * w:16 * w + 16], acc)
            else:
                t = w - NC
                s0 = 16 * NC + MOFF[t] // 8
                vg = [jnp.exp2(sv[pl.ds(VOFF[t] + 8 * g, 8), :]) for g in range(NVT[t] - 1, -1, -1)]
                acc = pv(B, j, t, vg + stream[s0:s0 + NMT[t]], acc)
            if w % NC == NC - 1:
                h, qi = uparams(j)
                (ota if w < NC else otb)[qi, h] = acc
                acc = None
        return carry

    for i, g in enumerate(qk(A, weights(A, 0), 0, L)):
        pc[pl.ds(8 * i, 8), :] = g
    for gi in range(NE):
        vpu_group(gi, 0, None, None)
    jax.lax.fori_loop(0, NU, body, 0)

    def slow(br):
        def unit(u, _):
            h, qi = uparams(u)
            kidx = h if br['a'] else 0
            w = jnp.concatenate([jnp.where(rows24 < DH, br['qt'][qi, h], 0.0),
                                 jnp.zeros((KW - HP, TQ), F32)], axis=0).astype(BF16)

            def scores(t):
                if br['a']:
                    k = pltpu.bitcast(
                        ka_scr[kidx, pl.ds(pl.multiple_of(t * (CK // 2), CK // 2), CK // 2), :], BF16)
                    s = jnp.dot(k, w, preferred_element_type=F32)
                    return jnp.concatenate([s[8 * g:8 * g + 8] for g in range(15, -1, -1)], axis=0)
                k = kbn_scr[pl.ds(pl.multiple_of(t * CK, CK), CK), :][:, :KW].astype(BF16)
                return jnp.dot(k, w, preferred_element_type=F32)

            m = jax.lax.fori_loop(
                0, NC, lambda t, m: jnp.maximum(m, jnp.max(scores(t), axis=0, keepdims=True)),
                jnp.full((1, TQ), -jnp.inf, F32))

            def acc_tile(t, acc):
                p = jnp.exp2(scores(t) - m)
                v = br['vt'][kidx, :, pl.ds(pl.multiple_of(t * CK, CK), CK)]
                return acc + jnp.dot(v, p, preferred_element_type=F32)
            br['ot'][qi, h] = jax.lax.fori_loop(0, NC, acc_tile, jnp.zeros((HP, TQ), F32))
            return 0
        jax.lax.fori_loop(0, NU, unit, 0)

    c_woa.wait()
    c_wob.wait()

    def ocp(qi, i):
        rows = pl.ds(mo(qi * TQ, TQ), TQ)
        return pltpu.make_async_copy(o_ref.at[i, rows, :], o_hbm.at[0, rows, pl.ds(i * D, D)],
                                     osem.at[2 * qi + i])

    def obody(qi, chk):
        lmin, lmax, bad = chk
        for i, (ot, wo_ref) in enumerate(((ota, woa_ref), (otb, wob_ref))):
            parts = []
            for h in range(H):
                a = ot[qi, h]
                lmin = jnp.minimum(lmin, a[16:24])
                lmax = jnp.maximum(lmax, a[16:24])
                l = ot[qi, h, pl.ds(DH, 1), :]
                r = pl.reciprocal(l, approx=True)
                r = r * (2.0 - l * r)
                parts.append((a * r)[:DH])
            o = jnp.concatenate(parts, axis=0).T.astype(BF16)
            y = jnp.dot(o, wo_ref[...], preferred_element_type=F32)
            nonfinite = jnp.where(jnp.abs(y) < 2.0 ** 127, 0.0, 1.0)
            bad = jnp.maximum(bad, jnp.max(nonfinite.reshape(TQ // 8, 8, D), axis=0))
            o_ref[i, pl.ds(pl.multiple_of(qi * TQ, TQ), TQ), :] = y.astype(o_ref.dtype)
            ocp(qi, i).start()
        return lmin, lmax, bad

    flag[0] = 1

    def attempt(p, _):
        @pl.when(flag[0] != 0)
        def _():
            @pl.when(p == 1)
            def _():
                slow(A)
                slow(B)
            one = jnp.ones((8, TQ), F32)
            lmin, lmax, bad = jax.lax.fori_loop(0, NQ, obody, (one, one, jnp.zeros((8, D), F32)))
            lok = jnp.logical_and(lmin[DH - 16:DH - 15] >= 1.0, lmax[DH - 16:DH - 15] < 2.0 ** 100)
            nbad = jnp.max(bad) + jnp.max(jnp.where(lok, 0.0, 1.0))
            flag[0] = jnp.where(nbad > 0.0, 1, 0)
            for qi in range(NQ):
                for i in range(2):
                    ocp(qi, i).wait()
        return 0
    jax.lax.fori_loop(0, 2, attempt, 0)


@jax.jit
def pallas_concat_heads__softmax_full_mha__grouped_kv_mqa__prompt_kernel(
    A_x: jax.Array,
    A_wqkv: jax.Array,
    A_wo: jax.Array,
    B_x: jax.Array,
    B_wq: jax.Array,
    B_wk: jax.Array,
    B_wv: jax.Array,
    B_wo: jax.Array,
):
    return pl.pallas_call(
        _kernel,
        in_specs=[pl.BlockSpec(memory_space=pl.ANY)] * 8,
        out_specs=pl.BlockSpec(memory_space=pl.ANY),
        out_shape=jax.ShapeDtypeStruct((1, S, 2 * D), BF16),
        scratch_shapes=[
            pltpu.VMEM((S, D), BF16),
            pltpu.VMEM((D, 3 * D), BF16),
            pltpu.VMEM((D, D), BF16),
            pltpu.VMEM((S, D), BF16),
            pltpu.VMEM((D, D), BF16),
            pltpu.VMEM((D, D), BF16),
            pltpu.VMEM((2, S, D), BF16),
            pltpu.SemaphoreType.DMA((7,)),
            pltpu.SemaphoreType.DMA((NQ,)),
            pltpu.SemaphoreType.DMA((2 * NQ,)),
            pltpu.VMEM((128, D), BF16),
            pltpu.VMEM((H, S // 2, KW), U32),
            pltpu.VMEM((1, S // 2, KW), U32),
            pltpu.VMEM((S, 128), F32),
            pltpu.VMEM((NQ, H, HP, TQ), F32),
            pltpu.VMEM((NQ, H, HP, TQ), F32),
            pltpu.VMEM((H, HP, S), F32),
            pltpu.VMEM((1, HP, S), F32),
            pltpu.VMEM((NQ, H, HP, TQ), F32),
            pltpu.VMEM((NQ, H, HP, TQ), F32),
            pltpu.VMEM((L, TQ), F32),
            pltpu.VMEM((768, TQ), F32),
            pltpu.VMEM((DH, 768, 128), F32),
            pltpu.VMEM((8, 128), jnp.int32),
            pltpu.VMEM((DH, D), BF16),
            pltpu.VMEM((DH, D), BF16),
            pltpu.SMEM((1,), jnp.int32),
        ],
        compiler_params=pltpu.CompilerParams(vmem_limit_bytes=110 * 1024 * 1024),
    )(A_x, A_wqkv, A_wo, B_x, B_wq, B_wk.T, B_wv.T, B_wo)
```
